```python
import jax
import jax.numpy as jnp

def _softmax(x, axis=-1):
    return jax.nn.softmax(x, axis=axis)
def _gelu(x):
    return jax.nn.gelu(x, approximate=True)
def _silu(x):
    return jax.nn.silu(x)
def _sigmoid(x):
    return jax.nn.sigmoid(x)
def _layernorm(x, axis=-1, eps=1e-5):
    m = jnp.mean(x, axis=axis, keepdims=True)
    v = jnp.var(x, axis=axis, keepdims=True)
    return (x - m) / jnp.sqrt(v + eps)
def _scatter_add(tgt, idx, src, axis=0):
    return tgt.at[idx].add(src)
def _segment_sum(src, seg, n):
    return jax.ops.segment_sum(src, seg, n)
class _Rng:
    def __init__(self, key):
        self._k = key
    def _next(self):
        self._k, sub = jax.random.split(self._k)
        return sub
    def normal(self, shape):
        return jax.random.normal(self._next(), shape, dtype=jnp.bfloat16)
    def randint(self, lo, hi, shape):
        return jax.random.randint(self._next(), shape, lo, hi, dtype=jnp.int32)
    def uniform(self, shape, lo=0.0, hi=1.0):
        return jax.random.uniform(self._next(), shape, jnp.bfloat16, lo, hi)
    def permutation(self, n):
        return jax.random.permutation(self._next(), n)


kernel_name = 'gated_mix__sliding_local_dilated__moe_arch_mod__prompt'

def setup_inputs():
    _rng = _Rng(jax.random.key(int.from_bytes(__import__("os").urandom(4), "little")))
    _w = (lambda a: (lambda t: t.astype(jnp.bfloat16) if jnp.issubdtype(t.dtype, jnp.floating) else t)(jnp.asarray(a)))
    def _A_setup():
        B, S, D = 1, 2048, 640
        return {
            "x": _w((lambda *s: _rng.normal(s) * 0.05)(B, S, D)),
            "wqkv": _w((lambda *s: _rng.normal(s) * 0.05)(D, 3 * D)),
            "wo": _w((lambda *s: _rng.normal(s) * 0.05)(D, D)),
        }
    _A_in = _A_setup()

    def _B_setup():
        B, S, D, F, C = 1, 2048, 640, 1728, 2
        return {
            "x": _w((lambda *s: _rng.normal(s) * 0.05)(B, S, D)),
            "w_r": _w((lambda *s: _rng.normal(s) * 0.05)(D)),
            "w_gate": _w((lambda *s: _rng.normal(s) * 0.05)(D, F)),
            "w_up": _w((lambda *s: _rng.normal(s) * 0.05)(D, F)),
            "w_down": _w((lambda *s: _rng.normal(s) * 0.05)(F, D)),
        }
    _B_in = _B_setup()

    return {
        "A_x": _A_in["x"],
        "A_wqkv": _A_in["wqkv"],
        "A_wo": _A_in["wo"],
        "B_x": _B_in["x"],
        "B_w_r": _B_in["w_r"],
        "B_w_gate": _B_in["w_gate"],
        "B_w_up": _B_in["w_up"],
        "B_w_down": _B_in["w_down"],
        "gate_w": _w((lambda *s: _rng.normal(s) * 0.05)(640)),
    }

def reference(A_x, A_wqkv, A_wo, B_x, B_w_r, B_w_gate, B_w_up, B_w_down, gate_w):
    def _A_ref(x, wqkv, wo):
        B, S, D = x.shape
        H = 32; Dh = D // H
        W, dil = 8, 2
        qkv = (lambda x, *d: x.transpose(*d))((x @ wqkv).reshape(B, S, 3, H, Dh), 2, 0, 3, 1, 4)
        q, k, v = qkv[0], qkv[1], qkv[2]
        scale = Dh ** -0.5
        pos = jnp.arange(S)
        off = jnp.arange(W) * dil
        idx = pos[:, None] - off[None, :]
        mask = idx >= 0
        idx_c = jnp.where(mask, idx, 0).reshape(-1)
        kg = k[:, :, idx_c, :].reshape(B, H, S, W, Dh)
        vg = v[:, :, idx_c, :].reshape(B, H, S, W, Dh)
        logits = jnp.einsum("bhsd,bhswd->bhsw", q, kg) * scale
        logits = jnp.where(mask[None, None, :, :], logits, -1e9)
        attn = _softmax(logits, axis=-1)
        o = jnp.einsum("bhsw,bhswd->bhsd", attn, vg)
        return (lambda x, *d: x.transpose(*d))(o, 0, 2, 1, 3).reshape(B, S, D) @ wo

    def _B_ref(x, w_r, w_gate, w_up, w_down):
        B, S, D = x.shape
        C = 2
        r = x @ w_r
        idx = jnp.argsort(-r, axis=-1)[:, :C]
        idx_e = jnp.repeat(idx.reshape(B, C, 1), D, axis=2)
        x_sel = jnp.take_along_axis(x, idx_e, axis=1)
        g = _silu(x_sel @ w_gate)
        u = x_sel @ w_up
        y = (g * u) @ w_down
        r_sel = _sigmoid(jnp.take_along_axis(r, idx, axis=1))
        y = y * r_sel.reshape(B, C, 1)
        b_off = (jnp.arange(B) * S).reshape(B, 1)
        flat_idx = (idx + b_off).reshape(B * C)
        zero = (x * 0.0).reshape(B * S, D)
        upd = _scatter_add(zero, flat_idx, y.reshape(B * C, D), axis=0)
        return x + upd.reshape(B, S, D)

    x = A_x
    g = _sigmoid((x * gate_w).sum(-1, keepdims=True))
    a = _A_ref(x, A_wqkv, A_wo)
    b = _B_ref(x, B_w_r, B_w_gate, B_w_up, B_w_down)
    return g * a + (1 - g) * b
```

```python
import functools

import jax
import jax.numpy as jnp
from jax import lax
import jax.experimental.pallas as pl
import jax.experimental.pallas.tpu as pltpu

S, D, F = 2048, 640, 1728
H, DH, WIN, DIL = 32, 20, 8, 2
NT = D // 128
HALO = 16
BM = 256
NB = S // BM
R = 16
EXP2_SCALE = (DH ** -0.5) * 1.4426950408889634
MASKED = -1e9 / (DH ** -0.5)

_NT_DIMS = (((1,), (1,)), ((), ()))
f32, bf16, u32, i32 = jnp.float32, jnp.bfloat16, jnp.uint32, jnp.int32


def _lanes(t):
    return slice(t * 128, (t + 1) * 128)


def _sigmoid(z):
    return 1.0 / (1.0 + jnp.exp(-z))


def _kernel(x_hbm, wqkv_hbm, wo_hbm, wr_hbm, wg_hbm, wu_hbm, wd_hbm, gw_hbm, out_hbm,
            x_v, wqkv_v, wo_v, wr_v, gw_v, wg_v, wu_v, wd_v,
            words, wt_s, wop_s, q_s, k_s, v_s, o_s, out_s, sems, osems):
    def cp(i, src, dst):
        return pltpu.make_async_copy(src, dst, sems.at[i])

    def rows(a, b):
        return pl.ds(a, b - a)

    c_x0 = cp(0, x_hbm.at[rows(0, BM)], x_v.at[rows(0, BM)])
    c_w = [cp(1 + p, wqkv_hbm.at[:, pl.ds(p * D, D)], wqkv_v.at[p]) for p in range(3)]
    c_x1 = cp(4, x_hbm.at[rows(BM, 2 * BM)], x_v.at[rows(BM, 2 * BM)])
    c_x2 = cp(5, x_hbm.at[rows(2 * BM, S)], x_v.at[rows(2 * BM, S)])
    c_wo = cp(6, wo_hbm, wo_v)
    c_wr = cp(7, wr_hbm, wr_v)
    c_gw = cp(8, gw_hbm, gw_v)
    c_wg = cp(9, wg_hbm, wg_v)
    c_wu = cp(10, wu_hbm, wu_v)
    c_wd = cp(11, wd_hbm, wd_v)

    def permute_rows(src_words, dst, row0, t):
        for j in range(DH // 2):
            w = src_words[pl.ds(j, H, stride=DH // 2), :]
            lo = pltpu.bitcast(w << 16, f32).astype(bf16)
            hi = pltpu.bitcast(w & jnp.uint32(0xFFFF0000), f32).astype(bf16)
            dst[pl.ds(row0 + 2 * j * H, H), _lanes(t)] = lo
            dst[pl.ds(row0 + (2 * j + 1) * H, H), _lanes(t)] = hi

    def prep_qkv(p):
        for t in range(NT):
            wt = wqkv_v[p, _lanes(t), :].T
            words[p * NT + t] = pltpu.bitcast(wt, u32)
            permute_rows(words.at[p * NT + t], wt_s, p * D, t)

    def prep_wo():
        for t in range(NT):
            words[3 * NT + t] = pltpu.bitcast(wo_v[:, _lanes(t)], u32)
            permute_rows(words.at[3 * NT + t], wop_s, 0, t)

    def proj(b, p):
        y = lax.dot_general(x_v[pl.ds(b * BM, BM), :], wt_s[pl.ds(p * D, D), :], _NT_DIMS,
                            preferred_element_type=f32)
        dst, off = ((q_s, 0), (k_s, HALO), (v_s, HALO))[p]
        for t in range(NT):
            dst[t, pl.ds(off + b * BM, BM), :] = y[:, _lanes(t)]
        if b == 0 and p == 1:
            for t in range(NT):
                k_s[t, pl.ds(0, HALO), :] = jnp.zeros((HALO, 128), f32)
        if b == 0 and p == 2:
            for t in range(NT):
                v_s[t, pl.ds(0, HALO), :] = jnp.broadcast_to(y[0:1, _lanes(t)], (HALO, 128))

    def attend(r0):
        q = [q_s[t, pl.ds(r0, R), :] for t in range(NT)]
        logits = []
        for w in range(WIN):
            base = HALO + r0 - DIL * w
            s = q[0] * k_s[0, pl.ds(base, R), :]
            for t in range(1, NT):
                s = s + q[t] * k_s[t, pl.ds(base, R), :]
            s = s + pltpu.roll(s, 64, 1)
            s = s + pltpu.roll(s, 32, 1)
            if r0 < DIL * w:
                pos = r0 + lax.broadcasted_iota(i32, (R, 128), 0)
                s = jnp.where(pos >= DIL * w, s, MASKED)
            logits.append(s)
        m = functools.reduce(jnp.maximum, logits)
        e = [jnp.exp2((s - m) * EXP2_SCALE) for s in logits]
        inv = 1.0 / functools.reduce(jnp.add, e)
        for t in range(NT):
            acc = e[0] * v_s[t, pl.ds(HALO + r0, R), :]
            for w in range(1, WIN):
                acc = acc + e[w] * v_s[t, pl.ds(HALO + r0 - DIL * w, R), :]
            o_s[pl.ds(r0, R), _lanes(t)] = (acc * inv).astype(bf16)

    def attend_part(b, part, nparts):
        n = BM // R // nparts
        for c in range(part * n, (part + 1) * n):
            attend(b * BM + c * R)

    def row_dot(x, w):
        s = x[:, _lanes(0)] * w[:, _lanes(0)]
        for t in range(1, NT):
            s = s + x[:, _lanes(t)] * w[:, _lanes(t)]
        return jnp.sum(s, axis=1, keepdims=True)

    def vec(ref):
        return ref[...].astype(f32).reshape(1, D)

    def mix(b):
        a = jnp.dot(o_s[pl.ds(b * BM, BM), :], wop_s[...], preferred_element_type=f32)
        x = x_v[pl.ds(b * BM, BM), :].astype(f32)
        g = _sigmoid(row_dot(x, vec(gw_v)))
        out_s[pl.ds(b * BM, BM), :] = (x + g * (a - x)).astype(bf16)

    def route():
        wr = vec(wr_v)
        lane = lax.broadcasted_iota(i32, (16, 128), 1)
        acc = jnp.zeros((16, 128), f32)
        for i in range(S // 16):
            r = row_dot(x_v[pl.ds(i * 16, 16), :].astype(f32), wr)
            acc = jnp.where(lane == i, r, acc)
        score = acc.astype(bf16).astype(f32)
        pos = lane * 16 + lax.broadcasted_iota(i32, (16, 128), 0)

        def best(sc):
            top = jnp.max(jnp.max(sc, axis=1, keepdims=True), axis=0, keepdims=True)
            cand = jnp.where(sc == top, pos, S - 1)
            return top, jnp.min(jnp.min(cand, axis=1, keepdims=True), axis=0, keepdims=True)

        r1, p1 = best(score)
        r2, p2 = best(jnp.where(pos == p1, -jnp.inf, score))
        return (p1[0, 0], p2[0, 0]), (r1, r2)

    def group(idx, lo, hi):
        return pl.multiple_of(jnp.clip(idx // 16, lo // 16, hi // 16 - 1) * 16, 16)

    def gather(idx):
        sel = []
        for j in range(2):
            g0 = group(idx[j], 0, S)
            xg = x_v[pl.ds(g0, 16), :].astype(f32)
            hit = lax.broadcasted_iota(i32, (16, D), 0) == idx[j] - g0
            sel.append(jnp.sum(jnp.where(hit, xg, 0.0), axis=0, keepdims=True))
        first = lax.broadcasted_iota(i32, (16, D), 0) == 0
        return jnp.where(first, sel[0], sel[1])

    def ffn(xs, top):
        xb = xs.astype(bf16)
        g = lax.dot_general(xb, wg_v[...], _NT_DIMS, preferred_element_type=f32)
        u = lax.dot_general(xb, wu_v[...], _NT_DIMS, preferred_element_type=f32)
        h = (g * _sigmoid(g) * u).astype(bf16)
        y = jnp.dot(h, wd_v[...], preferred_element_type=f32)
        first = lax.broadcasted_iota(i32, (16, 1), 0) == 0
        rs = _sigmoid(jnp.where(first, top[0], top[1]))
        gate = _sigmoid(row_dot(xs, vec(gw_v)))
        return y * (rs * (1.0 - gate))

    def patch(idx, delta, lo, hi):
        for j in range(2):
            g0 = group(idx[j], lo, hi)
            hit = lax.broadcasted_iota(i32, (16, D), 0) == idx[j] - g0
            cur = out_s[pl.ds(g0, 16), :].astype(f32)
            out_s[pl.ds(g0, 16), :] = jnp.where(hit, cur + delta[j:j + 1, :], cur).astype(bf16)

    def c_out(i, lo, hi):
        return pltpu.make_async_copy(out_s.at[rows(lo, hi)], out_hbm.at[rows(lo, hi)], osems.at[i])

    c_w[0].start(); c_x0.start(); c_w[1].start(); c_w[2].start()
    c_w[0].wait()
    c_x1.start(); c_wo.start(); c_gw.start(); c_wr.start()
    prep_qkv(0)
    c_x0.wait()
    c_w[1].wait()
    c_x2.start()
    prep_qkv(1)
    proj(0, 0)
    c_w[2].wait()
    c_wg.start(); c_wu.start(); c_wd.start()
    prep_qkv(2)
    proj(0, 1)
    proj(0, 2)
    c_x1.wait(); c_wo.wait(); c_gw.wait(); c_wr.wait()
    prep_wo()

    ROUTE_AT, FFN_AT = 2, 4
    outs = []
    for b in range(NB + 1):
        if b == 1:
            c_x2.wait()
        if b == FFN_AT:
            c_wg.wait(); c_wu.wait(); c_wd.wait()
        for p in range(3):
            if b + 1 < NB:
                proj(b + 1, p)
            if b < NB:
                attend_part(b, p, 4)
        if b >= 1:
            mix(b - 1)
        if b < NB:
            attend_part(b, 3, 4)
        if b == ROUTE_AT:
            idx, top = route()
            xs = gather(idx)
        if b == FFN_AT:
            delta = ffn(xs, top)
        if b >= FFN_AT:
            lo, hi = (0 if b == FFN_AT else (b - 1) * BM), b * BM
            patch(idx, delta, lo, hi)
            outs.append(c_out(len(outs), lo, hi))
            outs[-1].start()
    for c in outs:
        c.wait()


@jax.jit
def pallas_gated_mix__sliding_local_dilated__moe_arch_mod__prompt_kernel(
    A_x, A_wqkv, A_wo, B_x, B_w_r, B_w_gate, B_w_up, B_w_down, gate_w,
):
    del B_x
    hbm = pl.BlockSpec(memory_space=pl.ANY)
    vm = pltpu.VMEM
    out = pl.pallas_call(
        _kernel,
        in_specs=[hbm] * 8,
        out_specs=hbm,
        out_shape=jax.ShapeDtypeStruct((S, D), bf16),
        scratch_shapes=[
            vm((S, D), bf16), vm((3, D, D), bf16), vm((D, D), bf16), vm((D,), bf16), vm((D,), bf16),
            vm((F, D), bf16), vm((F, D), bf16), vm((F, D), bf16),
            vm((4 * NT, D // 2, 128), u32), vm((3 * D, D), bf16), vm((D, D), bf16),
            vm((NT, S, 128), f32), vm((NT, HALO + S, 128), f32), vm((NT, HALO + S, 128), f32),
            vm((S, D), bf16), vm((S, D), bf16),
            pltpu.SemaphoreType.DMA((12,)), pltpu.SemaphoreType.DMA((NB,)),
        ],
        compiler_params=pltpu.CompilerParams(vmem_limit_bytes=100 * 2 ** 20),
    )(A_x.reshape(S, D), A_wqkv, A_wo, B_w_r, B_w_gate.T, B_w_up.T, B_w_down, gate_w)
    return out.reshape(A_x.shape)
```

```python
import functools

import jax
import jax.numpy as jnp
from jax import lax
import jax.experimental.pallas as pl
import jax.experimental.pallas.tpu as pltpu

S, D, F = 2048, 640, 1728
H, DH, WIN, DIL = 32, 20, 8, 2
NT = D // 128
HALO = 16
BM = 256
NB = S // BM
R = 8
EXP2_SCALE = (DH ** -0.5) * 1.4426950408889634
MASKED = -1e9 / (DH ** -0.5)

STAGES = (
    "+q02 +q34 +x00 +x12 +k04 +v04 +x33 +gw +wr +wo +x47 +wg +wu +wd -q02 Wq02 -q34 Wq34 -x00 q0 -x12 q1 q2 -k04 -v04 -x33 Wk04 q3 Wv04 k0 v0",
    "-wo -gw -wr -x47 A0 sel0 Wo k1 v1 k2",
    "sel1 A1 v2 k3 v3",
    "-wg -wu up0 A2 q4 k4 v4 . up1 A3 M0 q5 k5 v5",
    "-wd down A4 M1 q6 k6 v6 . A5 M2 q7 k7",
    "O02 A6 M3 v7 M4",
    "O34 A7 M5 M6",
    "O56 M7 O77 -O02 -O34 -O56 -O77",
)
COPIES = [t[1:] for stage in STAGES for t in stage.split() if t[0] == "-"]
PIN = True
NPIN = 80
SLACK = 0
FLAGS = {"XLA_TPU_EVENLY_DISTRIBUTE_CRITICAL_NODES": True}
_NT_DIMS = (((1,), (1,)), ((), ()))
f32, bf16, u32, i32 = jnp.float32, jnp.bfloat16, jnp.uint32, jnp.int32


def _lanes(t):
    return slice(t * 128, (t + 1) * 128)


def _tree(op, xs):
    while len(xs) > 1:
        xs = [op(xs[i], xs[i + 1]) for i in range(0, len(xs), 2)]
    return xs[0]


def _sigmoid(z):
    return 1.0 / (1.0 + jnp.exp(-z))


def _kernel(x_hbm, wqkv_hbm, wo_hbm, wr_hbm, wg_hbm, wu_hbm, wd_hbm, gw_hbm, out_hbm,
            x_v, wqkv_v, wo_v, wr_v, gw_v, wg_v, wu_v, wd_v,
            words, wt_s, wop_s, qkv_s, o_bufs, out_s, h_s, xs_s, ys_s, top_s, idx_s, pins, sems):
    def rows(a, b):
        return pl.ds(a, b - a)

    def endpoints(name):
        if name[0] in "xO":
            r = rows(int(name[1]) * BM, (int(name[2]) + 1) * BM)
            if name[0] == "O":
                return out_s.at[r], out_hbm.at[r]
            r = rows(int(name[1]) * BM // 2, (int(name[2]) + 1) * BM // 2)
            return x_hbm.bitcast(u32).at[r], x_v.at[r]
        if name[0] in "qkv":
            p, r = "qkv".index(name[0]), rows(int(name[1]) * 128, (int(name[2]) + 1) * 128)
            return wqkv_hbm.at[r, pl.ds(p * D, D)], wqkv_v[p].at[r]
        return dict(wo=(wo_hbm, wo_v), wr=(wr_hbm, wr_v), gw=(gw_hbm, gw_v),
                    wg=(wg_hbm, wg_v), wu=(wu_hbm, wu_v), wd=(wd_hbm, wd_v))[name]

    copies = {name: pltpu.make_async_copy(*endpoints(name), sems.at[i]) for i, name in enumerate(COPIES)}

    def x_rows(r0, n, cols=slice(None)):
        return pltpu.bitcast(x_v[pl.ds(r0 // 2, n // 2), cols], bf16)

    def permute_rows(src_words, dst, t):
        for j in range(DH // 2):
            w = src_words[pl.ds(j, H, stride=DH // 2), :]
            lo = pltpu.bitcast(w << 16, f32).astype(bf16)
            hi = pltpu.bitcast(w & jnp.uint32(0xFFFF0000), f32).astype(bf16)
            dst[pl.ds(j * H, H // 2), _lanes(t)] = pltpu.bitcast(lo, u32)
            dst[pl.ds(j * H + H // 2, H // 2), _lanes(t)] = pltpu.bitcast(hi, u32)
        return pltpu.bitcast(hi, f32)[:8]

    def prep_qkv(p, lo, hi):
        for t in range(lo, hi + 1):
            wt = wqkv_v[p][_lanes(t), :].T
            words[p][t] = pltpu.bitcast(wt, u32)
            permute_rows(words[p].at[t], wt_s[p], t)

    def prep_wo():
        for t in range(NT):
            words[3][t] = pltpu.bitcast(wo_v[:, _lanes(t)], u32)
            yield permute_rows(words[3].at[t], wop_s, t)

    fillers = []

    paced = []
    clock = [0, 0, 0, 0]

    def matmul(tile):
        y = None
        for k in range(NT):
            y = tile(k) if y is None else y + tile(k)
            clock[3] += 1
            if clock[3] % 4 == 0:
                for _ in range(min(4, len(fillers))):
                    fillers.pop(0)()
        clock[0] += 1
        for item in paced:
            gen, total, done = item
            want = min(total, -(-total * clock[0] // max(clock[1] - SLACK, 1)))
            last = None
            for _ in range(want - done):
                last = next(gen)
            item[2] = want
            if last is not None and PIN:
                pin = pins[clock[2]]
                clock[2] += 1
                pin[...] = last
                pin[...] = y[-8:]
        return y

    def proj(b, p):
        cur = qkv_s[b][p]
        for t in range(NT):
            yt = matmul(lambda k: lax.dot_general(
                x_rows(b * BM, BM, _lanes(k)), pltpu.bitcast(wt_s[p][pl.ds(t * 64, 64), _lanes(k)], bf16),
                _NT_DIMS, preferred_element_type=f32))
            if p == 0:
                cur[t] = yt
                continue
            cur[t, pl.ds(HALO, BM), :] = yt
            if b == 0:
                cur[t, pl.ds(0, HALO), :] = (jnp.zeros((HALO, 128), f32) if p == 1 else
                                             jnp.broadcast_to(yt[0:1], (HALO, 128)))
            if b + 1 < NB:
                qkv_s[b + 1][p][t, pl.ds(0, HALO), :] = yt[BM - HALO:]

    def attend(b):
        q_s, k_s, v_s = qkv_s[b]
        o_s = o_bufs[b]

        def scores(i):
            q = [q_s[t, pl.ds(i * R, R), :] for t in range(NT)]
            out = []
            for w in range(WIN):
                base = HALO + i * R - DIL * w
                s = q[0] * k_s[0, pl.ds(base, R), :]
                for t in range(1, NT):
                    s = s + q[t] * k_s[t, pl.ds(base, R), :]
                out.append((s, pltpu.roll(s, 64, 1)))
            return out

        def fold(i, parts):
            out = []
            for s, r in parts:
                s = s + r
                out.append((s, pltpu.roll(s, 32, 1)))
            return out

        def softmax(i, parts):
            logits = []
            for w, (s, r) in enumerate(parts):
                s = s + r
                if b * BM + i * R < DIL * w:
                    pos = b * BM + i * R + lax.broadcasted_iota(i32, (R, 128), 0)
                    s = jnp.where(pos >= DIL * w, s, MASKED)
                logits.append(s)
            m = _tree(jnp.maximum, logits)
            e = [jnp.exp2((s - m) * EXP2_SCALE) for s in logits]
            den = _tree(jnp.add, e)
            return e, den, pl.reciprocal(den, approx=True)

        def values(i, parts):
            e, den, inv = parts
            inv = inv * (2.0 - den * inv)
            out = []
            for t in range(NT):
                acc = e[0] * v_s[t, pl.ds(HALO + i * R, R), :]
                for w in range(1, WIN):
                    acc = acc + e[w] * v_s[t, pl.ds(HALO + i * R - DIL * w, R), :]
                out.append(acc * inv)
            return out

        n = BM // R
        per = 16 // R if R < 16 else 1
        st = [{} for _ in range(4)]
        for c in range(n + 3):
            if c < n:
                st[0][c] = scores(c)
                last = st[0][c][-1][0]
            if 0 <= c - 1 < n:
                st[1][c - 1] = fold(c - 1, st[0].pop(c - 1))
            if 0 <= c - 2 < n:
                st[2][c - 2] = softmax(c - 2, st[1].pop(c - 2))
            if 0 <= c - 3 < n:
                i = c - 3
                st[3][i] = values(i, st[2].pop(i))
                last = st[3][i][-1]
                if (i + 1) % per == 0:
                    done = [st[3].pop(j) for j in range(i + 1 - per, i + 1)]
                    r0 = (i + 1 - per) * R
                    for t in range(NT):
                        o = jnp.concatenate([d[t] for d in done], axis=0).astype(bf16)
                        o_s[pl.ds(r0 // 2, per * R // 2), _lanes(t)] = pltpu.bitcast(o, u32)
            yield last[:8]

    def row_dot(x, w):
        s = x[:, _lanes(0)] * w[:, _lanes(0)]
        for t in range(1, NT):
            s = s + x[:, _lanes(t)] * w[:, _lanes(t)]
        return jnp.sum(s, axis=1, keepdims=True)

    def vec(ref):
        return ref[...].astype(f32).reshape(1, D)

    def mix(b):
        g = _sigmoid(row_dot(x_rows(b * BM, BM).astype(f32), vec(gw_v)))
        for t in range(NT):
            a = matmul(lambda k: jnp.dot(
                pltpu.bitcast(o_bufs[b][:, _lanes(k)], bf16),
                pltpu.bitcast(wop_s[pl.ds(k * 64, 64), _lanes(t)], bf16), preferred_element_type=f32))
            x = x_rows(b * BM, BM, _lanes(t)).astype(f32)
            out_s[pl.ds(b * BM, BM), _lanes(t)] = (x + g * (a - x)).astype(bf16)

    def route(part):
        wr = vec(wr_v)
        lane = lax.broadcasted_iota(i32, (16, 128), 1)
        acc = jnp.zeros((16, 128), f32) if part == 0 else top_s[...]
        for i in range(part * S // 32, (part + 1) * S // 32):
            r = row_dot(x_rows(i * 16, 16).astype(f32), wr)
            acc = jnp.where(lane == i, r, acc)
            if i % 8 == 7:
                yield acc[:8]
        if part == 0:
            top_s[...] = acc
            return
        score = acc.astype(bf16).astype(f32)
        pos = lane * 16 + lax.broadcasted_iota(i32, (16, 128), 0)

        def best(sc):
            top = jnp.max(jnp.max(sc, axis=1, keepdims=True), axis=0, keepdims=True)
            cand = jnp.where(sc == top, pos, S - 1)
            return top, jnp.min(jnp.min(cand, axis=1, keepdims=True), axis=0, keepdims=True)

        r1, p1 = best(score)
        r2, p2 = best(jnp.where(pos == p1, -jnp.inf, score))
        idx, top = (p1[0, 0], p2[0, 0]), (r1, r2)
        idx_s[0] = idx[0]
        idx_s[1] = idx[1]
        first = lax.broadcasted_iota(i32, (16, 128), 0) == 0
        top_s[...] = jnp.where(first, top[0], top[1])
        xs = gather(idx)
        xs_s[...] = xs
        yield xs[:8, :128]

    def group(idx, lo, hi):
        return pl.multiple_of(jnp.clip(idx // 16, lo // 16, hi // 16 - 1) * 16, 16)

    def gather(idx):
        sel = []
        for j in range(2):
            g0 = group(idx[j], 0, S)
            xg = pltpu.bitcast(x_v[pl.ds(pl.multiple_of(g0 // 2, 8), 8), :], bf16).astype(f32)
            hit = lax.broadcasted_iota(i32, (16, D), 0) == idx[j] - g0
            sel.append(jnp.sum(jnp.where(hit, xg, 0.0), axis=0, keepdims=True))
        first = lax.broadcasted_iota(i32, (16, D), 0) == 0
        return jnp.where(first, sel[0], sel[1])

    f_tiles = [(n, min(128, F - n)) for n in range(0, F, 128)]

    def ffn_up(part, parts):
        xb = xs_s[...].astype(bf16)
        acc = {}

        def tile(w_v, n, w, k):
            y = lax.dot_general(xb[:, _lanes(k)], w_v[pl.ds(n, w), _lanes(k)], _NT_DIMS, preferred_element_type=f32)
            key = w_v is wu_v
            acc[key] = y if k == 0 else acc[key] + y
            if key and k == NT - 1:
                g = acc[False]
                h_s[:, pl.ds(n, w)] = (g * _sigmoid(g) * acc[True]).astype(bf16)

        per = -(-len(f_tiles) // parts)
        for n, w in f_tiles[part * per:(part + 1) * per]:
            for w_v in (wg_v, wu_v):
                fillers.extend(functools.partial(tile, w_v, n, w, k) for k in range(NT))

    def ffn_down():
        acc = {}

        def tile(t, n, w):
            y = jnp.dot(h_s[:, pl.ds(n, w)], wd_v[pl.ds(n, w), _lanes(t)], preferred_element_type=f32)
            acc[t] = y if n == 0 else acc[t] + y
            if n + w == F:
                ys_s[:, _lanes(t)] = acc[t] * scale

        gate = _sigmoid(row_dot(xs_s[...], vec(gw_v)))
        scale = _sigmoid(top_s[...]) * (1.0 - gate)
        for t in range(NT):
            fillers.extend(functools.partial(tile, t, n, w) for n, w in f_tiles)

    def patch(lo, hi):
        idx, delta = (idx_s[0], idx_s[1]), ys_s[...]
        for j in range(2):
            g0 = group(idx[j], lo, hi)
            hit = lax.broadcasted_iota(i32, (16, D), 0) == idx[j] - g0
            cur = out_s[pl.ds(g0, 16), :].astype(f32)
            out_s[pl.ds(g0, 16), :] = jnp.where(hit, cur + delta[j:j + 1, :], cur).astype(bf16)

    def run(task):
        if task == ".":
            while fillers:
                fillers.pop(0)()
            for gen, _, _ in paced:
                for _ in gen:
                    pass
            paced.clear()
        elif task[0] == "+":
            copies[task[1:]].start()
        elif task[0] == "-":
            copies[task[1:]].wait()
        elif task[0] in "qkv":
            proj(int(task[1]), "qkv".index(task[0]))
        elif task[0] == "A":
            paced.append([attend(int(task[1])), BM // R + 3, 0])
        elif task[0] == "M":
            mix(int(task[1]))
        elif task[0] == "W":
            if task[1] == "o":
                paced.append([prep_wo(), NT, 0])
            else:
                prep_qkv("qkv".index(task[1]), int(task[2]), int(task[3]))
        elif task[0] == "O":
            patch(int(task[1]) * BM, (int(task[2]) + 1) * BM)
            copies[task].start()
        else:
            dict(sel0=lambda: paced.append([route(0), S // 256, 0]),
                 sel1=lambda: paced.append([route(1), S // 256 + 1, 0]), up0=lambda: ffn_up(0, 2), up1=lambda: ffn_up(1, 2), down=ffn_down)[task]()

    step = pl.program_id(0)
    for i, stage in enumerate(STAGES):
        @pl.when(step == i)
        def _(i=i, stage=stage):
            with jax.named_scope(f"stage{i}"):
                clock[2:] = [0, 0]
                for phase in stage.split(" . "):
                    clock[:2] = [0, NT * sum(t[0] in "qkvM" for t in phase.split())]
                    for task in phase.split() + ["."]:
                        run(task)
                assert not fillers and not paced


@jax.jit
def pallas_gated_mix__sliding_local_dilated__moe_arch_mod__prompt_kernel(
    A_x, A_wqkv, A_wo, B_x, B_w_r, B_w_gate, B_w_up, B_w_down, gate_w,
):
    del B_x
    hbm = pl.BlockSpec(memory_space=pl.ANY)
    vm = pltpu.VMEM
    out = pl.pallas_call(
        _kernel,
        grid=(len(STAGES),),
        in_specs=[hbm] * 8,
        out_specs=hbm,
        out_shape=jax.ShapeDtypeStruct((S, D), bf16),
        scratch_shapes=[
            vm((S // 2, D), u32), [vm((D, D), bf16)] * 3, vm((D, D), bf16), vm((D,), bf16), vm((D,), bf16),
            vm((F, D), bf16), vm((F, D), bf16), vm((F, D), bf16),
            [vm((NT, D // 2, 128), u32)] * 4, [vm((D // 2, D), u32)] * 3, vm((D // 2, D), u32),
            [[vm((NT, BM, 128), f32), vm((NT, HALO + BM, 128), f32), vm((NT, HALO + BM, 128), f32)]] * NB,
            [vm((BM // 2, D), u32)] * NB, vm((S, D), bf16), vm((16, F), bf16),
            vm((16, D), f32), vm((16, D), f32), vm((16, 128), f32), pltpu.SMEM((2,), i32), [vm((8, 128), f32)] * NPIN,
            pltpu.SemaphoreType.DMA((len(COPIES),)),
        ],
        compiler_params=pltpu.CompilerParams(vmem_limit_bytes=100 * 2 ** 20, flags=FLAGS,
                                             dimension_semantics=("arbitrary",)),
    )(A_x.reshape(S, D), A_wqkv, A_wo, B_w_r, B_w_gate.T, B_w_up.T, B_w_down, gate_w)
    return out.reshape(A_x.shape)
```

```python
import functools

import jax
import jax.numpy as jnp
from jax import lax
import jax.experimental.pallas as pl
import jax.experimental.pallas.tpu as pltpu

S, D, F = 2048, 640, 1728
H, DH, WIN, DIL = 32, 20, 8, 2
NT = D // 128
HALO = 16
BM = 256
NB = S // BM
R = 8
EXP2_SCALE = (DH ** -0.5) * 1.4426950408889634
MASKED = -1e9 / (DH ** -0.5)

STAGES = (
    "+q02 +q34 +x00 +x12 +k04 +v04 +x33 +gw +wr +wo +x47 +wg +wu +wd -q02 Wq02 -q34 Wq34 -x00 q0",
    "-x12 q1 q2",
    "-k04 -v04 -x33 Wk04 q3 Wv04 k0 v0",
    "-wo -gw -wr A0 sel0 Wo k1 v1 k2",
    "-x47 sel1 A1 v2 k3 v3",
    "-wg -wu up A2 q4 k4 v4 . A3 M0 q5 k5 v5",
    "-wd down A4 M1 q6 k6 v6 . A5 M2 q7 k7",
    "O02 A6 M3 v7 M4",
    "O34 A7 M5 O55 M6 O66 . T7 -O02 -O34 -O55 -O66 -T70 -T71 -T72 -T73 -T74",
)
COPIES = [t[1:] for stage in STAGES for t in stage.split() if t[0] == "-"]
PIN = True
NPIN = 80
SLACK = 0
FLAGS = {"XLA_TPU_EVENLY_DISTRIBUTE_CRITICAL_NODES": True}
_NT_DIMS = (((1,), (1,)), ((), ()))
f32, bf16, u32, i32 = jnp.float32, jnp.bfloat16, jnp.uint32, jnp.int32


def _lanes(t):
    return slice(t * 128, (t + 1) * 128)


def _tree(op, xs):
    while len(xs) > 1:
        xs = [op(xs[i], xs[i + 1]) for i in range(0, len(xs), 2)]
    return xs[0]


def _sigmoid(z):
    return 1.0 / (1.0 + jnp.exp(-z))


def _kernel(x_hbm, wqkv_hbm, wo_hbm, wr_hbm, wg_hbm, wu_hbm, wd_hbm, gw_hbm, out_hbm,
            x_v, wqkv_v, wo_v, wr_v, gw_v, wg_v, wu_v, wd_v,
            words, wt_s, wop_s, qkv_s, o_bufs, out_s, h_s, xs_s, ys_s, top_s, idx_s, pins, sems):
    def rows(a, b):
        return pl.ds(a, b - a)

    def endpoints(name):
        if name[0] in "xO":
            r = rows(int(name[1]) * BM, (int(name[2]) + 1) * BM)
            if name[0] == "O":
                return out_s.at[r], out_hbm.at[r]
            r = rows(int(name[1]) * BM // 2, (int(name[2]) + 1) * BM // 2)
            return x_hbm.bitcast(u32).at[r], x_v.at[r]
        if name[0] == "T":
            r, c = pl.ds(int(name[1]) * BM, BM), pl.ds(int(name[2]) * 128, 128)
            return out_s.at[r, c], out_hbm.at[r, c]
        if name[0] in "qkv":
            p, r = "qkv".index(name[0]), rows(int(name[1]) * 128, (int(name[2]) + 1) * 128)
            return wqkv_hbm.at[r, pl.ds(p * D, D)], wqkv_v[p].at[r]
        return dict(wo=(wo_hbm, wo_v), wr=(wr_hbm, wr_v), gw=(gw_hbm, gw_v),
                    wg=(wg_hbm, wg_v), wu=(wu_hbm, wu_v), wd=(wd_hbm, wd_v))[name]

    copies = {name: pltpu.make_async_copy(*endpoints(name), sems.at[i]) for i, name in enumerate(COPIES)}

    def x_rows(r0, n, cols=slice(None)):
        return pltpu.bitcast(x_v[pl.ds(r0 // 2, n // 2), cols], bf16)

    def permute_rows(src_words, dst, t):
        for j in range(DH // 2):
            w = src_words[pl.ds(j, H, stride=DH // 2), :]
            lo = pltpu.bitcast(w << 16, f32).astype(bf16)
            hi = pltpu.bitcast(w & jnp.uint32(0xFFFF0000), f32).astype(bf16)
            dst[pl.ds(j * H, H // 2), _lanes(t)] = pltpu.bitcast(lo, u32)
            dst[pl.ds(j * H + H // 2, H // 2), _lanes(t)] = pltpu.bitcast(hi, u32)
        return pltpu.bitcast(hi, f32)[:8]

    def prep_qkv(p, lo, hi):
        for t in range(lo, hi + 1):
            wt = wqkv_v[p][_lanes(t), :].T
            words[p][t] = pltpu.bitcast(wt, u32)
            permute_rows(words[p].at[t], wt_s[p], t)

    def prep_wo():
        for t in range(NT):
            words[3][t] = pltpu.bitcast(wo_v[:, _lanes(t)], u32)
            yield permute_rows(words[3].at[t], wop_s, t)

    fillers = []

    paced = []
    clock = [0, 0, 0, 0]

    def matmul(tile):
        y = None
        for k in range(NT):
            y = tile(k) if y is None else y + tile(k)
            clock[3] += 1
            if clock[3] % 4 == 0 and k > 0:
                for _ in range(min(4, len(fillers))):
                    fillers.pop(0)()
        clock[0] += 1
        for item in paced:
            gen, total, done = item
            want = min(total, -(-total * clock[0] // max(clock[1] - SLACK, 1)))
            last = None
            for _ in range(want - done):
                last = next(gen)
            item[2] = want
            if last is not None and PIN:
                pin = pins[clock[2]]
                clock[2] += 1
                pin[...] = last
                pin[...] = y[-8:]
        return y

    def proj(b, p):
        cur = qkv_s[b][p]
        for t in range(NT):
            yt = matmul(lambda k: lax.dot_general(
                x_rows(b * BM, BM, _lanes(k)), pltpu.bitcast(wt_s[p][pl.ds(t * 64, 64), _lanes(k)], bf16),
                _NT_DIMS, preferred_element_type=f32))
            if p == 0:
                cur[t] = yt
                continue
            cur[t, pl.ds(HALO, BM), :] = yt
            if b == 0:
                cur[t, pl.ds(0, HALO), :] = (jnp.zeros((HALO, 128), f32) if p == 1 else
                                             jnp.broadcast_to(yt[0:1], (HALO, 128)))
            if b + 1 < NB:
                qkv_s[b + 1][p][t, pl.ds(0, HALO), :] = yt[BM - HALO:]

    def attend(b):
        q_s, k_s, v_s = qkv_s[b]
        o_s = o_bufs[b]

        def scores(i):
            q = [q_s[t, pl.ds(i * R, R), :] for t in range(NT)]
            out = []
            for w in range(WIN):
                base = HALO + i * R - DIL * w
                s = q[0] * k_s[0, pl.ds(base, R), :]
                for t in range(1, NT):
                    s = s + q[t] * k_s[t, pl.ds(base, R), :]
                out.append((s, pltpu.roll(s, 64, 1)))
            return out

        def fold(i, parts):
            out = []
            for s, r in parts:
                s = s + r
                out.append((s, pltpu.roll(s, 32, 1)))
            return out

        def softmax(i, parts):
            logits = []
            for w, (s, r) in enumerate(parts):
                s = s + r
                if b * BM + i * R < DIL * w:
                    pos = b * BM + i * R + lax.broadcasted_iota(i32, (R, 128), 0)
                    s = jnp.where(pos >= DIL * w, s, MASKED)
                logits.append(s)
            m = _tree(jnp.maximum, logits)
            e = [jnp.exp2((s - m) * EXP2_SCALE) for s in logits]
            den = _tree(jnp.add, e)
            return e, den, pl.reciprocal(den, approx=True)

        def values(i, parts):
            e, den, inv = parts
            inv = inv * (2.0 - den * inv)
            out = []
            for t in range(NT):
                acc = e[0] * v_s[t, pl.ds(HALO + i * R, R), :]
                for w in range(1, WIN):
                    acc = acc + e[w] * v_s[t, pl.ds(HALO + i * R - DIL * w, R), :]
                out.append(acc * inv)
            return out

        n = BM // R
        per = 16 // R if R < 16 else 1
        st = [{} for _ in range(4)]
        for c in range(n + 3):
            if c < n:
                st[0][c] = scores(c)
                last = st[0][c][-1][0]
            if 0 <= c - 1 < n:
                st[1][c - 1] = fold(c - 1, st[0].pop(c - 1))
            if 0 <= c - 2 < n:
                st[2][c - 2] = softmax(c - 2, st[1].pop(c - 2))
            if 0 <= c - 3 < n:
                i = c - 3
                st[3][i] = values(i, st[2].pop(i))
                last = st[3][i][-1]
                if (i + 1) % per == 0:
                    done = [st[3].pop(j) for j in range(i + 1 - per, i + 1)]
                    r0 = (i + 1 - per) * R
                    for t in range(NT):
                        o = jnp.concatenate([d[t] for d in done], axis=0).astype(bf16)
                        o_s[pl.ds(r0 // 2, per * R // 2), _lanes(t)] = pltpu.bitcast(o, u32)
            yield last[:8]

    def row_dot(x, w):
        s = x[:, _lanes(0)] * w[:, _lanes(0)]
        for t in range(1, NT):
            s = s + x[:, _lanes(t)] * w[:, _lanes(t)]
        return jnp.sum(s, axis=1, keepdims=True)

    def vec(ref):
        return ref[...].astype(f32).reshape(1, D)

    def mix(b, tiled_out=False):
        g = _sigmoid(row_dot(x_rows(b * BM, BM).astype(f32), vec(gw_v)))
        for t in range(NT):
            a = matmul(lambda k: jnp.dot(
                pltpu.bitcast(o_bufs[b][:, _lanes(k)], bf16),
                pltpu.bitcast(wop_s[pl.ds(k * 64, 64), _lanes(t)], bf16), preferred_element_type=f32))
            x = x_rows(b * BM, BM, _lanes(t)).astype(f32)
            out_s[pl.ds(b * BM, BM), _lanes(t)] = (x + g * (a - x)).astype(bf16)
            if tiled_out:
                patch(b * BM, (b + 1) * BM, _lanes(t))
                copies[f"T{b}{t}"].start()

    def route(part):
        wr = vec(wr_v)
        lane = lax.broadcasted_iota(i32, (16, 128), 1)
        acc = jnp.zeros((16, 128), f32) if part == 0 else top_s[...]
        for i in range(part * S // 32, (part + 1) * S // 32):
            r = row_dot(x_rows(i * 16, 16).astype(f32), wr)
            acc = jnp.where(lane == i, r, acc)
            if i % 8 == 7:
                yield acc[:8]
        if part == 0:
            top_s[...] = acc
            return
        score = acc.astype(bf16).astype(f32)
        pos = lane * 16 + lax.broadcasted_iota(i32, (16, 128), 0)

        def best(sc):
            top = jnp.max(jnp.max(sc, axis=1, keepdims=True), axis=0, keepdims=True)
            cand = jnp.where(sc == top, pos, S - 1)
            return top, jnp.min(jnp.min(cand, axis=1, keepdims=True), axis=0, keepdims=True)

        r1, p1 = best(score)
        r2, p2 = best(jnp.where(pos == p1, -jnp.inf, score))
        idx, top = (p1[0, 0], p2[0, 0]), (r1, r2)
        idx_s[0] = idx[0]
        idx_s[1] = idx[1]
        first = lax.broadcasted_iota(i32, (16, 128), 0) == 0
        top_s[...] = jnp.where(first, top[0], top[1])
        xs = gather(idx)
        xs_s[...] = xs
        yield xs[:8, :128]

    def group(idx, lo, hi):
        return pl.multiple_of(jnp.clip(idx // 16, lo // 16, hi // 16 - 1) * 16, 16)

    def gather(idx):
        sel = []
        for j in range(2):
            g0 = group(idx[j], 0, S)
            xg = pltpu.bitcast(x_v[pl.ds(pl.multiple_of(g0 // 2, 8), 8), :], bf16).astype(f32)
            hit = lax.broadcasted_iota(i32, (16, D), 0) == idx[j] - g0
            sel.append(jnp.sum(jnp.where(hit, xg, 0.0), axis=0, keepdims=True))
        first = lax.broadcasted_iota(i32, (16, D), 0) == 0
        return jnp.where(first, sel[0], sel[1])

    f_tiles = [(n, min(128, F - n)) for n in range(0, F, 128)]

    def ffn_up(part, parts):
        xb = xs_s[...].astype(bf16)
        acc = {}

        def tile(w_v, n, w, k):
            y = lax.dot_general(xb[:, _lanes(k)], w_v[pl.ds(n, w), _lanes(k)], _NT_DIMS, preferred_element_type=f32)
            key = w_v is wu_v
            acc[key] = y if k == 0 else acc[key] + y
            if key and k == NT - 1:
                g = acc[False]
                h_s[:, pl.ds(n, w)] = (g * _sigmoid(g) * acc[True]).astype(bf16)

        per = -(-len(f_tiles) // parts)
        for n, w in f_tiles[part * per:(part + 1) * per]:
            for w_v in (wg_v, wu_v):
                fillers.extend(functools.partial(tile, w_v, n, w, k) for k in range(NT))

    def ffn_down():
        acc = {}

        def tile(t, n, w):
            y = jnp.dot(h_s[:, pl.ds(n, w)], wd_v[pl.ds(n, w), _lanes(t)], preferred_element_type=f32)
            acc[t] = y if n == 0 else acc[t] + y
            if n + w == F:
                ys_s[:, _lanes(t)] = acc[t] * scale

        gate = _sigmoid(row_dot(xs_s[...], vec(gw_v)))
        scale = _sigmoid(top_s[...]) * (1.0 - gate)
        for t in range(NT):
            fillers.extend(functools.partial(tile, t, n, w) for n, w in f_tiles)

    def patch(lo, hi, cols=slice(0, D)):
        idx, delta = (idx_s[0], idx_s[1]), ys_s[:, cols]
        for j in range(2):
            g0 = group(idx[j], lo, hi)
            hit = lax.broadcasted_iota(i32, (16, cols.stop - cols.start), 0) == idx[j] - g0
            cur = out_s[pl.ds(g0, 16), cols].astype(f32)
            out_s[pl.ds(g0, 16), cols] = jnp.where(hit, cur + delta[j:j + 1, :], cur).astype(bf16)

    def run(task):
        if task == ".":
            for gen, _, _ in paced:
                for _ in gen:
                    pass
            paced.clear()
        elif task[0] == "+":
            copies[task[1:]].start()
        elif task[0] == "-":
            copies[task[1:]].wait()
        elif task[0] in "qkv":
            proj(int(task[1]), "qkv".index(task[0]))
        elif task[0] == "A":
            paced.append([attend(int(task[1])), BM // R + 3, 0])
        elif task[0] in "MT":
            mix(int(task[1]), task[0] == "T")
        elif task[0] == "W":
            if task[1] == "o":
                paced.append([prep_wo(), NT, 0])
            else:
                prep_qkv("qkv".index(task[1]), int(task[2]), int(task[3]))
        elif task[0] == "O":
            patch(int(task[1]) * BM, (int(task[2]) + 1) * BM)
            copies[task].start()
        else:
            dict(sel0=lambda: paced.append([route(0), S // 256, 0]),
                 sel1=lambda: paced.append([route(1), S // 256 + 1, 0]), up=lambda: ffn_up(0, 1), down=ffn_down)[task]()

    step = pl.program_id(0)
    for i, stage in enumerate(STAGES):
        @pl.when(step * (i + 2) < 1)
        def _(i=i, stage=stage):
            with jax.named_scope(f"stage{i}"):
                clock[2:] = [0, 0]
                for phase in stage.split(" . "):
                    clock[:2] = [0, NT * sum(t[0] in "qkvMT" for t in phase.split())]
                    for task in phase.split() + ["."]:
                        run(task)
                while fillers:
                    fillers.pop(0)()


@jax.jit
def pallas_gated_mix__sliding_local_dilated__moe_arch_mod__prompt_kernel(
    A_x, A_wqkv, A_wo, B_x, B_w_r, B_w_gate, B_w_up, B_w_down, gate_w,
):
    del B_x
    hbm = pl.BlockSpec(memory_space=pl.ANY)
    vm = pltpu.VMEM
    out = pl.pallas_call(
        _kernel,
        grid=(2,),
        in_specs=[hbm] * 8,
        out_specs=hbm,
        out_shape=jax.ShapeDtypeStruct((S, D), bf16),
        scratch_shapes=[
            vm((S // 2, D), u32), [vm((D, D), bf16)] * 3, vm((D, D), bf16), vm((D,), bf16), vm((D,), bf16),
            vm((F, D), bf16), vm((F, D), bf16), vm((F, D), bf16),
            [vm((NT, D // 2, 128), u32)] * 4, [vm((D // 2, D), u32)] * 3, vm((D // 2, D), u32),
            [[vm((NT, BM, 128), f32), vm((NT, HALO + BM, 128), f32), vm((NT, HALO + BM, 128), f32)]] * NB,
            [vm((BM // 2, D), u32)] * NB, vm((S, D), bf16), vm((16, F), bf16),
            vm((16, D), f32), vm((16, D), f32), vm((16, 128), f32), pltpu.SMEM((2,), i32), [vm((8, 128), f32)] * NPIN,
            pltpu.SemaphoreType.DMA((len(COPIES),)),
        ],
        compiler_params=pltpu.CompilerParams(vmem_limit_bytes=100 * 2 ** 20, flags=FLAGS,
                                             dimension_semantics=("arbitrary",)),
    )(A_x.reshape(S, D), A_wqkv, A_wo, B_w_r, B_w_gate.T, B_w_up.T, B_w_down, gate_w)
    return out.reshape(A_x.shape)
```

```python
import functools

import jax
import jax.numpy as jnp
from jax import lax
import jax.experimental.pallas as pl
import jax.experimental.pallas.tpu as pltpu

S, D, F = 2048, 640, 1728
H, DH, WIN, DIL = 32, 20, 8, 2
NT = D // 128
HALO = 16
BM = 256
NB = S // BM
R = 8
EXP2_SCALE = (DH ** -0.5) * 1.4426950408889634
MASKED = -1e9 / (DH ** -0.5)

STAGES = (
    "+gw +wr +q02 +q34 +x00 +x12 +k04 +v04 +x33 -q02 Wq02 -q34 Wq34 -x00 -gw -wr G0 q0",
    "-x12 G1 G2 q1 q2",
    "-k04 -v04 -x33 +wo +x47 +wg R3 Wk04 q3 Wv04 k0 v0",
    "-x47 +wu +wd A0 R4 R5 R6 R7 k1 v1 k2",
    "route K3 K4 A1 v2 k3 v3",
    "-wg -wu -wo up A2 Wo q4 k4 v4 . A3 M0 q5 k5 v5",
    "-wd down A4 K5 q6 k6 v6 . A5 K6 M1 q7 k7",
    "O01 A6 K7 M2 v7 M3 . O23 A72 M4 M5 O45 M6 . O66 T7 -O01 -O23 -O45 -O66 -T70 -T71 -T72 -T73 -T74",
)
COPIES = [t[1:] for stage in STAGES for t in stage.split() if t[0] == "-"]
LAG = (0, 1, 2, 3)
PIN = True
NPIN = 120
SLACK = 2
FLAGS = {"XLA_TPU_EVENLY_DISTRIBUTE_CRITICAL_NODES": True}
_NT_DIMS = (((1,), (1,)), ((), ()))
f32, bf16, u32, i32 = jnp.float32, jnp.bfloat16, jnp.uint32, jnp.int32


def _lanes(t):
    return slice(t * 128, (t + 1) * 128)


def _tree(op, xs):
    while len(xs) > 1:
        xs = [op(xs[i], xs[i + 1]) for i in range(0, len(xs), 2)]
    return xs[0]


def _sigmoid(z):
    return 1.0 / (1.0 + jnp.exp(-z))


def _kernel(x_hbm, wqkv_hbm, wo_hbm, wr_hbm, wg_hbm, wu_hbm, wd_hbm, gw_hbm, out_hbm,
            x_v, wqkv_v, wo_v, wr_v, gw_v, wg_v, wu_v, wd_v,
            words, wt_s, wop_s, qkv_s, o_bufs, out_s, h_s, g_s, keep_s, score_s, xs_s, ys_s, top_s, idx_s, pins, sems):
    def rows(a, b):
        return pl.ds(a, b - a)

    def endpoints(name):
        if name[0] in "xO":
            r = rows(int(name[1]) * BM, (int(name[2]) + 1) * BM)
            if name[0] == "O":
                return out_s.at[r], out_hbm.at[r]
            r = rows(int(name[1]) * BM // 2, (int(name[2]) + 1) * BM // 2)
            return x_hbm.bitcast(u32).at[r], x_v.at[r]
        if name[0] == "T":
            r, c = pl.ds(int(name[1]) * BM, BM), pl.ds(int(name[2]) * 128, 128)
            return out_s.at[r, c], out_hbm.at[r, c]
        if name[0] in "qkv":
            p, r = "qkv".index(name[0]), rows(int(name[1]) * 128, (int(name[2]) + 1) * 128)
            return wqkv_hbm.at[r, pl.ds(p * D, D)], wqkv_v[p].at[r]
        return dict(wo=(wo_hbm, wo_v), wr=(wr_hbm, wr_v), gw=(gw_hbm, gw_v),
                    wg=(wg_hbm, wg_v), wu=(wu_hbm, wu_v), wd=(wd_hbm, wd_v))[name]

    copies = {name: pltpu.make_async_copy(*endpoints(name), sems.at[i]) for i, name in enumerate(COPIES)}

    def x_rows(r0, n, cols=slice(None)):
        return pltpu.bitcast(x_v[pl.ds(r0 // 2, n // 2), cols], bf16)

    def permute_rows(src_words, dst, t):
        for j in range(DH // 2):
            w = src_words[pl.ds(j, H, stride=DH // 2), :]
            lo = pltpu.bitcast(w << 16, f32).astype(bf16)
            hi = pltpu.bitcast(w & jnp.uint32(0xFFFF0000), f32).astype(bf16)
            dst[pl.ds(j * H, H // 2), _lanes(t)] = pltpu.bitcast(lo, u32)
            dst[pl.ds(j * H + H // 2, H // 2), _lanes(t)] = pltpu.bitcast(hi, u32)
        return pltpu.bitcast(hi, f32)[:8]

    def prep_qkv(p, lo, hi):
        for t in range(lo, hi + 1):
            wt = wqkv_v[p][_lanes(t), :].T
            words[p][t] = pltpu.bitcast(wt, u32)
            permute_rows(words[p].at[t], wt_s[p], t)

    def prep_wo():
        for t in range(NT):
            w = pltpu.bitcast(wo_v[:, _lanes(t)], u32)
            words[3][t] = w
            yield pltpu.bitcast(w[-8:], f32)
            yield permute_rows(words[3].at[t], wop_s, t)

    fillers = []

    paced = []
    clock = [0, 0, 0, 0]

    def matmul(tile):
        y = None
        for k in range(NT):
            y = tile(k) if y is None else y + tile(k)
            clock[3] += 1
            if clock[3] % 4 == 0 and k > 0:
                for _ in range(min(4, len(fillers))):
                    fillers.pop(0)()
        clock[0] += 1
        for item in paced:
            gen, total, done, slack = item
            want = min(total, -(-total * clock[0] // max(clock[1] - slack, 1)))
            last = None
            for _ in range(want - done):
                last = next(gen)
            item[2] = want
            if last is not None and PIN:
                pin = pins[clock[2]]
                clock[2] += 1
                pin[...] = last
                pin[...] = y[-8:]
        return y

    def proj(b, p):
        cur = qkv_s[b][p]
        for t in range(NT):
            yt = matmul(lambda k: lax.dot_general(
                x_rows(b * BM, BM, _lanes(k)), pltpu.bitcast(wt_s[p][pl.ds(t * 64, 64), _lanes(k)], bf16),
                _NT_DIMS, preferred_element_type=f32))
            if p == 0:
                cur[t] = yt
                continue
            cur[t, pl.ds(HALO, BM), :] = yt
            if b == 0:
                cur[t, pl.ds(0, HALO), :] = (jnp.zeros((HALO, 128), f32) if p == 1 else
                                             jnp.broadcast_to(yt[0:1], (HALO, 128)))
            if b + 1 < NB:
                qkv_s[b + 1][p][t, pl.ds(0, HALO), :] = yt[BM - HALO:]

    def attend(b):
        q_s, k_s, v_s = qkv_s[b]
        o_s = o_bufs[b]

        def scores(i):
            q = [q_s[t, pl.ds(i * R, R), :] for t in range(NT)]
            out = []
            for w in range(WIN):
                base = HALO + i * R - DIL * w
                s = q[0] * k_s[0, pl.ds(base, R), :]
                for t in range(1, NT):
                    s = s + q[t] * k_s[t, pl.ds(base, R), :]
                out.append((s, pltpu.roll(s, 64, 1)))
            return out

        def fold(i, parts):
            out = []
            for s, r in parts:
                s = s + r
                out.append((s, pltpu.roll(s, 32, 1)))
            return out

        def softmax(i, parts):
            logits = []
            for w, (s, r) in enumerate(parts):
                s = s + r
                if b * BM + i * R < DIL * w:
                    pos = b * BM + i * R + lax.broadcasted_iota(i32, (R, 128), 0)
                    s = jnp.where(pos >= DIL * w, s, MASKED)
                logits.append(s)
            m = _tree(jnp.maximum, logits)
            e = [jnp.exp2((s - m) * EXP2_SCALE) for s in logits]
            den = _tree(jnp.add, e)
            return e, den, pl.reciprocal(den, approx=True)

        def values(i, parts):
            e, den, inv = parts
            inv = inv * (2.0 - den * inv)
            out = []
            for t in range(NT):
                acc = e[0] * v_s[t, pl.ds(HALO + i * R, R), :]
                for w in range(1, WIN):
                    acc = acc + e[w] * v_s[t, pl.ds(HALO + i * R - DIL * w, R), :]
                out.append(acc * inv)
            return out

        n = BM // R
        per = 16 // R if R < 16 else 1
        st = [{} for _ in range(4)]
        for c in range(n + LAG[3]):
            if c < n:
                st[0][c] = scores(c)
                last = st[0][c][-1][0]
            if 0 <= c - LAG[1] < n:
                st[1][c - LAG[1]] = fold(c - LAG[1], st[0].pop(c - LAG[1]))
            if 0 <= c - LAG[2] < n:
                st[2][c - LAG[2]] = softmax(c - LAG[2], st[1].pop(c - LAG[2]))
                last = st[2][c - LAG[2]][1]
            if 0 <= c - LAG[3] < n:
                i = c - LAG[3]
                st[3][i] = values(i, st[2].pop(i))
                last = st[3][i][-1]
                if (i + 1) % per == 0:
                    done = [st[3].pop(j) for j in range(i + 1 - per, i + 1)]
                    r0 = (i + 1 - per) * R
                    for t in range(NT):
                        o = jnp.concatenate([d[t] for d in done], axis=0).astype(bf16)
                        o_s[pl.ds(r0 // 2, per * R // 2), _lanes(t)] = pltpu.bitcast(o, u32)
            yield last[:8]

    def row_dot(x, w):
        s = x[:, _lanes(0)] * w[:, _lanes(0)]
        for t in range(1, NT):
            s = s + x[:, _lanes(t)] * w[:, _lanes(t)]
        return jnp.sum(s, axis=1, keepdims=True)

    def vec(ref):
        return ref[...].astype(f32).reshape(1, D)

    def mix(b, tiled_out=False):
        for t in range(NT):
            a = matmul(lambda k: jnp.dot(
                pltpu.bitcast(o_bufs[b][:, _lanes(k)], bf16),
                pltpu.bitcast(wop_s[pl.ds(k * 64, 64), _lanes(t)], bf16), preferred_element_type=f32))
            out_s[pl.ds(b * BM, BM), _lanes(t)] = (g_s[b][...] * a + keep_s[b][t]).astype(bf16)
            if tiled_out:
                patch(b * BM, (b + 1) * BM, _lanes(t))
                copies[f"T{b}{t}"].start()

    def gates(b, mixing, routing):
        gw, wr = vec(gw_v), vec(wr_v)
        lane = lax.broadcasted_iota(i32, (16, 128), 1)
        acc = jnp.zeros((16, 128), f32)
        for i in range(BM // 16):
            x = x_rows(b * BM + i * 16, 16).astype(f32)
            if mixing:
                g = _sigmoid(row_dot(x, gw))
                g_s[b][pl.ds(i * 16, 16), :] = last = jnp.broadcast_to(g, (16, 128))
                for t in range(NT):
                    keep_s[b][t, pl.ds(i * 16, 16), :] = (1.0 - g) * x[:, _lanes(t)]
            if routing:
                acc = last = jnp.where(lane == b * (BM // 16) + i, row_dot(x, wr), acc)
                if i == BM // 16 - 1:
                    score_s[b][...] = acc
            if i % 2:
                yield last[:8]

    def route():
        lane = lax.broadcasted_iota(i32, (16, 128), 1)
        acc = score_s[0][...]
        for b in range(1, NB):
            acc = jnp.where(lane >= b * (BM // 16), score_s[b][...], acc)
        score = acc.astype(bf16).astype(f32)
        pos = lane * 16 + lax.broadcasted_iota(i32, (16, 128), 0)

        def best(sc):
            top = jnp.max(jnp.max(sc, axis=1, keepdims=True), axis=0, keepdims=True)
            cand = jnp.where(sc == top, pos, S - 1)
            return top, jnp.min(jnp.min(cand, axis=1, keepdims=True), axis=0, keepdims=True)

        r1, p1 = best(score)
        r2, p2 = best(jnp.where(pos == p1, -jnp.inf, score))
        idx, top = (p1[0, 0], p2[0, 0]), (r1, r2)
        idx_s[0] = idx[0]
        idx_s[1] = idx[1]
        first = lax.broadcasted_iota(i32, (16, 128), 0) == 0
        top_s[...] = jnp.where(first, top[0], top[1])
        xs = gather(idx)
        xs_s[...] = xs
        yield xs[:8, :128]

    def group(idx, lo, hi):
        return pl.multiple_of(jnp.clip(idx // 16, lo // 16, hi // 16 - 1) * 16, 16)

    def gather(idx):
        sel = []
        for j in range(2):
            g0 = group(idx[j], 0, S)
            xg = pltpu.bitcast(x_v[pl.ds(pl.multiple_of(g0 // 2, 8), 8), :], bf16).astype(f32)
            hit = lax.broadcasted_iota(i32, (16, D), 0) == idx[j] - g0
            sel.append(jnp.sum(jnp.where(hit, xg, 0.0), axis=0, keepdims=True))
        first = lax.broadcasted_iota(i32, (16, D), 0) == 0
        return jnp.where(first, sel[0], sel[1])

    f_tiles = [(n, min(128, F - n)) for n in range(0, F, 128)]

    def ffn_up(lo, hi):
        xb = xs_s[...].astype(bf16)
        acc = {}

        def tile(w_v, n, w, k):
            y = lax.dot_general(xb[:, _lanes(k)], w_v[pl.ds(n, w), _lanes(k)], _NT_DIMS, preferred_element_type=f32)
            key = w_v is wu_v
            acc[key] = y if k == 0 else acc[key] + y
            if key and k == NT - 1:
                g = acc[False]
                h_s[:, pl.ds(n, w)] = (g * _sigmoid(g) * acc[True]).astype(bf16)

        for n, w in f_tiles[lo:hi]:
            for w_v in (wg_v, wu_v):
                fillers.extend(functools.partial(tile, w_v, n, w, k) for k in range(NT))

    def ffn_down():
        acc = {}

        def tile(t, n, w):
            y = jnp.dot(h_s[:, pl.ds(n, w)], wd_v[pl.ds(n, w), _lanes(t)], preferred_element_type=f32)
            acc[t] = y if n == 0 else acc[t] + y
            if n + w == F:
                ys_s[:, _lanes(t)] = acc[t] * scale

        gate = _sigmoid(row_dot(xs_s[...], vec(gw_v)))
        scale = _sigmoid(top_s[...]) * (1.0 - gate)
        for t in range(NT):
            fillers.extend(functools.partial(tile, t, n, w) for n, w in f_tiles)

    def patch(lo, hi, cols=slice(0, D)):
        idx, delta = (idx_s[0], idx_s[1]), ys_s[:, cols]
        for j in range(2):
            g0 = group(idx[j], lo, hi)
            hit = lax.broadcasted_iota(i32, (16, cols.stop - cols.start), 0) == idx[j] - g0
            cur = out_s[pl.ds(g0, 16), cols].astype(f32)
            out_s[pl.ds(g0, 16), cols] = jnp.where(hit, cur + delta[j:j + 1, :], cur).astype(bf16)

    def run(task):
        if task == ".":
            for gen, *_ in paced:
                for _ in gen:
                    pass
            paced.clear()
        elif task[0] == "+":
            copies[task[1:]].start()
        elif task[0] == "-":
            copies[task[1:]].wait()
        elif task[0] in "qkv":
            proj(int(task[1]), "qkv".index(task[0]))
        elif task[0] in "GKR":
            paced.append([gates(int(task[1]), task[0] != "R", task[0] != "K"), BM // 32, 0, int(task[2:] or 0)])
        elif task[0] == "A":
            paced.append([attend(int(task[1])), BM // R + LAG[3], 0, int(task[2:] or 0)])
        elif task[0] in "MT":
            mix(int(task[1]), task[0] == "T")
        elif task[0] == "W":
            if task[1] == "o":
                paced.append([prep_wo(), 2 * NT, 0, 0])
            else:
                prep_qkv("qkv".index(task[1]), int(task[2]), int(task[3]))
        elif task[0] == "O":
            patch(int(task[1]) * BM, (int(task[2]) + 1) * BM)
            copies[task].start()
        else:
            dict(route=lambda: [None for _ in route()], up=lambda: ffn_up(0, 14), up0=lambda: ffn_up(0, 12), up1=lambda: ffn_up(12, 14), down=ffn_down)[task]()

    step = pl.program_id(0)
    for i, stage in enumerate(STAGES):
        @pl.when(step * (i + 2) < 1)
        def _(i=i, stage=stage):
            with jax.named_scope(f"stage{i}"):
                clock[2:] = [0, 0]
                for phase in stage.split(" . "):
                    clock[:2] = [0, NT * sum(t[0] in "qkvMT" for t in phase.split())]
                    for task in phase.split() + ["."]:
                        run(task)
                while fillers:
                    fillers.pop(0)()


@jax.jit
def pallas_gated_mix__sliding_local_dilated__moe_arch_mod__prompt_kernel(
    A_x, A_wqkv, A_wo, B_x, B_w_r, B_w_gate, B_w_up, B_w_down, gate_w,
):
    del B_x
    hbm = pl.BlockSpec(memory_space=pl.ANY)
    vm = pltpu.VMEM
    out = pl.pallas_call(
        _kernel,
        grid=(2,),
        in_specs=[hbm] * 8,
        out_specs=hbm,
        out_shape=jax.ShapeDtypeStruct((S, D), bf16),
        scratch_shapes=[
            vm((S // 2, D), u32), [vm((D, D), bf16)] * 3, vm((D, D), bf16), vm((D,), bf16), vm((D,), bf16),
            vm((F, D), bf16), vm((F, D), bf16), vm((F, D), bf16),
            [vm((NT, D // 2, 128), u32)] * 4, [vm((D // 2, D), u32)] * 3, vm((D // 2, D), u32),
            [[vm((NT, BM, 128), f32), vm((NT, HALO + BM, 128), f32), vm((NT, HALO + BM, 128), f32)]] * NB,
            [vm((BM // 2, D), u32)] * NB, vm((S, D), bf16), vm((16, F), bf16),
            [vm((BM, 128), f32)] * NB, [vm((NT, BM, 128), f32)] * NB, [vm((16, 128), f32)] * NB,
            vm((16, D), f32), vm((16, D), f32), vm((16, 128), f32), pltpu.SMEM((2,), i32), [vm((8, 128), f32)] * NPIN,
            pltpu.SemaphoreType.DMA((len(COPIES),)),
        ],
        compiler_params=pltpu.CompilerParams(vmem_limit_bytes=100 * 2 ** 20, flags=FLAGS,
                                             dimension_semantics=("arbitrary",)),
    )(A_x.reshape(S, D), A_wqkv, A_wo, B_w_r, B_w_gate.T, B_w_up.T, B_w_down, gate_w)
    return out.reshape(A_x.shape)
```

```python
import functools

import jax
import jax.numpy as jnp
from jax import lax
import jax.experimental.pallas as pl
import jax.experimental.pallas.tpu as pltpu

S, D, F = 2048, 640, 1728
H, DH, WIN, DIL = 32, 20, 8, 2
NT = D // 128
HALO = 16
BM = 256
NB = S // BM
R = 8
EXP2_SCALE = (DH ** -0.5) * 1.4426950408889634
MASKED = -1e9 * 1.4426950408889634

STAGES = (
    "+q02 +q34 +x00 +x13 +gw +wr +k04 +v04 -q02 Wq02 -q34 Wq34 -x00 q0",
    "-x13 -gw -wr G0 G1 q1 q2",
    "-k04 -v04 +wo +x47 +wg G2 R3 Wk04 q3 Wv04 k0 v0",
    "-x47 +wu +wd R4 R5 R6 R7 . A0 k1 v1 k2",
    "route . K3 K4 A1 v2 k3 v3",
    "-wg -wu -wo Wo q4 . up A2 k4 v4 q5 . A3 M0 k5 v5",
    "-wd down A4 K5 q6 k6 v6 . A5 K6 M1 q7 k7",
    "O01 A6 K7 v7 M2 M3 . O23 A74 M4 O44 M5 O55 M6 . O66 T7 -O01 -O23 -O44 -O55 -O66 -T70 -T71 -T72 -T73 -T74",
)
COPIES = [t[1:] for stage in STAGES for t in stage.split() if t[0] == "-"]
assert all(t[1:] in COPIES for stage in STAGES for t in stage.split() if t[0] == "+")
FLAGS = {"XLA_TPU_EVENLY_DISTRIBUTE_CRITICAL_NODES": True}
_NT_DIMS = (((1,), (1,)), ((), ()))
f32, bf16, u32, i32 = jnp.float32, jnp.bfloat16, jnp.uint32, jnp.int32


def _lanes(t):
    return slice(t * 128, (t + 1) * 128)


def _tree(op, xs):
    while len(xs) > 1:
        xs = [op(xs[i], xs[i + 1]) for i in range(0, len(xs), 2)]
    return xs[0]


def _sigmoid(z):
    return 1.0 / (1.0 + jnp.exp(-z))


def _kernel(x_hbm, wqkv_hbm, wo_hbm, wr_hbm, wg_hbm, wu_hbm, wd_hbm, gw_hbm, out_hbm,
            x_v, wqkv_v, wo_v, wr_v, gw_v, wg_v, wu_v, wd_v,
            words, wt_s, wop_s, qkv_s, o_bufs, out_s, h_s, g_s, keep_s, score_s, xs_s, ys_s, top_s, idx_s, sems):
    def rows(a, b):
        return pl.ds(a, b - a)

    def endpoints(name):
        if name[0] in "xO":
            r = rows(int(name[1]) * BM, (int(name[2]) + 1) * BM)
            if name[0] == "O":
                return out_s.at[r], out_hbm.at[r]
            r = rows(int(name[1]) * BM // 2, (int(name[2]) + 1) * BM // 2)
            return x_hbm.bitcast(u32).at[r], x_v.at[r]
        if name[0] == "T":
            r, c = pl.ds(int(name[1]) * BM, BM), pl.ds(int(name[2]) * 128, 128)
            return out_s.at[r, c], out_hbm.at[r, c]
        if name[0] in "qkv":
            p, r = "qkv".index(name[0]), rows(int(name[1]) * 128, (int(name[2]) + 1) * 128)
            return wqkv_hbm.at[r, pl.ds(p * D, D)], wqkv_v[p].at[r]
        return dict(wo=(wo_hbm, wo_v), wr=(wr_hbm, wr_v), gw=(gw_hbm, gw_v),
                    wg=(wg_hbm, wg_v), wu=(wu_hbm, wu_v), wd=(wd_hbm, wd_v))[name]

    copies = {name: pltpu.make_async_copy(*endpoints(name), sems.at[i]) for i, name in enumerate(COPIES)}

    def x_rows(r0, n, cols=slice(None)):
        return pltpu.bitcast(x_v[pl.ds(r0 // 2, n // 2), cols], bf16)

    def permute_rows(src_words, dst, t):
        for j in range(DH // 2):
            w = src_words[pl.ds(j, H, stride=DH // 2), :]
            lo = pltpu.bitcast(w << 16, f32).astype(bf16)
            hi = pltpu.bitcast(w & jnp.uint32(0xFFFF0000), f32).astype(bf16)
            dst[pl.ds(j * H, H // 2), _lanes(t)] = pltpu.bitcast(lo, u32)
            dst[pl.ds(j * H + H // 2, H // 2), _lanes(t)] = pltpu.bitcast(hi, u32)

    def prep_qkv(p, lo, hi):
        for t in range(lo, hi + 1):
            wt = wqkv_v[p][_lanes(t), :].T
            words[p][t, pl.ds(0, D // 2), :] = pltpu.bitcast(wt, u32)
            permute_rows(words[p].at[t], wt_s[p], t)

    def prep_wo():
        for t in range(NT):
            words[3][t, pl.ds(0, D // 2), :] = pltpu.bitcast(wo_v[:, _lanes(t)], u32)
            yield
            yield permute_rows(words[3].at[t], wop_s, t)

    fillers = []

    paced = []
    clock = [0, 0, 0]

    def matmul(tile):
        y = None
        for k in range(NT):
            y = tile(k) if y is None else y + tile(k)
            clock[2] += 1
            if clock[2] % 4 == 0 and k > 0:
                for _ in range(min(4, len(fillers))):
                    fillers.pop(0)()
        clock[0] += 1
        for item in paced:
            gen, total, done, slack = item
            item[2] = min(total, -(-total * clock[0] // max(clock[1] - slack, 1)))
            for _ in range(item[2] - done):
                next(gen)
        return y

    def proj(b, p):
        cur = qkv_s[b][p]
        for t in range(NT):
            yt = matmul(lambda k: lax.dot_general(
                x_rows(b * BM, BM, _lanes(k)), pltpu.bitcast(wt_s[p][pl.ds(t * 64, 64), _lanes(k)], bf16),
                _NT_DIMS, preferred_element_type=f32))
            if p == 0:
                cur[t] = yt
                continue
            cur[t, pl.ds(HALO, BM), :] = yt
            if b == 0:
                cur[t, pl.ds(0, HALO), :] = (jnp.zeros((HALO, 128), f32) if p == 1 else
                                             jnp.broadcast_to(yt[0:1], (HALO, 128)))
            if b + 1 < NB:
                qkv_s[b + 1][p][t, pl.ds(0, HALO), :] = yt[BM - HALO:]

    def attend(b):
        q_s, k_s, v_s = qkv_s[b]
        o_s = o_bufs[b]

        def scores(i):
            q = [q_s[t, pl.ds(i * R, R), :] * EXP2_SCALE for t in range(NT)]
            out = []
            for w in range(WIN):
                base = HALO + i * R - DIL * w
                s = q[0] * k_s[0, pl.ds(base, R), :]
                for t in range(1, NT):
                    s = s + q[t] * k_s[t, pl.ds(base, R), :]
                out.append((s, pltpu.roll(s, 64, 1)))
            return out

        def fold(parts):
            out = []
            for s, r in parts:
                s = s + r
                out.append((s, pltpu.roll(s, 32, 1)))
            return out

        def softmax(i, parts):
            logits = []
            for w, (s, r) in enumerate(parts):
                s = s + r
                if b * BM + i * R < DIL * w:
                    pos = b * BM + i * R + lax.broadcasted_iota(i32, (R, 128), 0)
                    s = jnp.where(pos >= DIL * w, s, MASKED)
                logits.append(s)
            m = _tree(jnp.maximum, logits)
            e = [jnp.exp2(s - m) for s in logits]
            den = _tree(jnp.add, e)
            return e, den, pl.reciprocal(den, approx=True)

        def values(i, parts):
            e, den, inv = parts
            inv = inv * (2.0 - den * inv)
            out = []
            for t in range(NT):
                acc = e[0] * v_s[t, pl.ds(HALO + i * R, R), :]
                for w in range(1, WIN):
                    acc = acc + e[w] * v_s[t, pl.ds(HALO + i * R - DIL * w, R), :]
                out.append(acc * inv)
            return out

        n = BM // R
        st = [{} for _ in range(4)]
        for c in range(n + 3):
            if c < n:
                st[0][c] = scores(c)
            if 0 <= c - 1 < n:
                st[1][c - 1] = fold(st[0].pop(c - 1))
            if 0 <= c - 2 < n:
                st[2][c - 2] = softmax(c - 2, st[1].pop(c - 2))
            if 0 <= c - 3 < n:
                i = c - 3
                st[3][i] = values(i, st[2].pop(i))
                if i % 2:
                    lo, hi = st[3].pop(i - 1), st[3].pop(i)
                    for t in range(NT):
                        o = jnp.concatenate([lo[t], hi[t]], axis=0).astype(bf16)
                        o_s[pl.ds((i - 1) * R // 2, R), _lanes(t)] = pltpu.bitcast(o, u32)
            yield

    def row_dot(x, w):
        s = x[:, _lanes(0)] * w[:, _lanes(0)]
        for t in range(1, NT):
            s = s + x[:, _lanes(t)] * w[:, _lanes(t)]
        return jnp.sum(s, axis=1, keepdims=True)

    def vec(ref):
        return ref[...].astype(f32).reshape(1, D)

    def mix(b, tiled_out=False):
        for t in range(NT):
            a = matmul(lambda k: jnp.dot(
                pltpu.bitcast(o_bufs[b][:, _lanes(k)], bf16),
                pltpu.bitcast(wop_s[pl.ds(k * 64, 64), _lanes(t)], bf16), preferred_element_type=f32))
            out_s[pl.ds(b * BM, BM), _lanes(t)] = (g_s[b][...] * a + keep_s[b][t]).astype(bf16)
            if tiled_out:
                patch(b * BM, (b + 1) * BM, _lanes(t))
                copies[f"T{b}{t}"].start()

    def gates(b, mixing, routing):
        gw, wr = vec(gw_v), vec(wr_v)
        lane = lax.broadcasted_iota(i32, (16, 128), 1)
        acc = jnp.zeros((16, 128), f32)
        for i in range(BM // 16):
            x = x_rows(b * BM + i * 16, 16).astype(f32)
            if mixing:
                g = _sigmoid(row_dot(x, gw))
                g_s[b][pl.ds(i * 16, 16), :] = jnp.broadcast_to(g, (16, 128))
                for t in range(NT):
                    keep_s[b][t, pl.ds(i * 16, 16), :] = (1.0 - g) * x[:, _lanes(t)]
            if routing:
                acc = jnp.where(lane == b * (BM // 16) + i, row_dot(x, wr), acc)
                if i == BM // 16 - 1:
                    score_s[b][...] = acc
            if i % 2:
                yield

    def route():
        lane = lax.broadcasted_iota(i32, (16, 128), 1)
        acc = score_s[0][...]
        for b in range(1, NB):
            acc = jnp.where(lane >= b * (BM // 16), score_s[b][...], acc)
        score = acc.astype(bf16).astype(f32)
        pos = lane * 16 + lax.broadcasted_iota(i32, (16, 128), 0)

        def best(sc, taken):
            top = jnp.max(jnp.max(sc, axis=1, keepdims=True), axis=0, keepdims=True)
            cand = jnp.where((sc == top) & (pos != taken), pos, S - 1)
            return top, jnp.min(jnp.min(cand, axis=1, keepdims=True), axis=0, keepdims=True)

        r1, p1 = best(score, -1)
        r2, p2 = best(jnp.where(pos == p1, -jnp.inf, score), p1)
        idx, top = (p1[0, 0], p2[0, 0]), (r1, r2)
        idx_s[0] = idx[0]
        idx_s[1] = idx[1]
        first = lax.broadcasted_iota(i32, (16, 128), 0) == 0
        top_s[...] = jnp.where(first, top[0], top[1])
        xs = gather(idx)
        xs_s[...] = xs

    def group(idx, lo, hi):
        return pl.multiple_of(jnp.clip(idx // 16, lo // 16, hi // 16 - 1) * 16, 16)

    def gather(idx):
        sel = []
        for j in range(2):
            g0 = group(idx[j], 0, S)
            xg = pltpu.bitcast(x_v[pl.ds(pl.multiple_of(g0 // 2, 8), 8), :], bf16).astype(f32)
            hit = lax.broadcasted_iota(i32, (16, D), 0) == idx[j] - g0
            sel.append(jnp.sum(jnp.where(hit, xg, 0.0), axis=0, keepdims=True))
        first = lax.broadcasted_iota(i32, (16, D), 0) == 0
        return jnp.where(first, sel[0], sel[1])

    f_tiles = [(n, min(128, F - n)) for n in range(0, F, 128)]

    def ffn_up():
        xb = xs_s[...].astype(bf16)
        acc = {}

        def tile(w_v, n, w, k):
            y = lax.dot_general(xb[:, _lanes(k)], w_v[pl.ds(n, w), _lanes(k)], _NT_DIMS, preferred_element_type=f32)
            key = w_v is wu_v
            acc[key] = y if k == 0 else acc[key] + y
            if key and k == NT - 1:
                g = acc[False]
                h_s[:, pl.ds(n, w)] = (g * _sigmoid(g) * acc[True]).astype(bf16)

        for n, w in f_tiles:
            for w_v in (wg_v, wu_v):
                fillers.extend(functools.partial(tile, w_v, n, w, k) for k in range(NT))

    def ffn_down():
        acc = {}

        def tile(t, n, w):
            y = jnp.dot(h_s[:, pl.ds(n, w)], wd_v[pl.ds(n, w), _lanes(t)], preferred_element_type=f32)
            acc[t] = y if n == 0 else acc[t] + y
            if n + w == F:
                ys_s[:, _lanes(t)] = acc[t] * scale

        gate = _sigmoid(row_dot(xs_s[...], vec(gw_v)))
        scale = _sigmoid(top_s[...]) * (1.0 - gate)
        for t in range(NT):
            fillers.extend(functools.partial(tile, t, n, w) for n, w in f_tiles)

    def patch(lo, hi, cols=slice(0, D)):
        idx, delta = (idx_s[0], idx_s[1]), ys_s[:, cols]
        for j in range(2):
            g0 = group(idx[j], lo, hi)
            hit = lax.broadcasted_iota(i32, (16, cols.stop - cols.start), 0) == idx[j] - g0
            cur = out_s[pl.ds(g0, 16), cols].astype(f32)
            out_s[pl.ds(g0, 16), cols] = jnp.where(hit, cur + delta[j:j + 1, :], cur).astype(bf16)

    def run(task):
        if task == ".":
            for gen, *_ in paced:
                for _ in gen:
                    pass
            paced.clear()
        elif task[0] == "+":
            copies[task[1:]].start()
        elif task[0] == "-":
            copies[task[1:]].wait()
        elif task[0] in "qkv":
            proj(int(task[1]), "qkv".index(task[0]))
        elif task[0] in "GKR":
            paced.append([gates(int(task[1]), task[0] != "R", task[0] != "K"), BM // 32, 0, int(task[2:] or 0)])
        elif task[0] == "A":
            paced.append([attend(int(task[1])), BM // R + 3, 0, int(task[2:] or 0)])
        elif task[0] in "MT":
            mix(int(task[1]), task[0] == "T")
        elif task[0] == "W":
            if task[1] == "o":
                paced.append([prep_wo(), 2 * NT, 0, 0])
            else:
                prep_qkv("qkv".index(task[1]), int(task[2]), int(task[3]))
        elif task[0] == "O":
            patch(int(task[1]) * BM, (int(task[2]) + 1) * BM)
            copies[task].start()
        else:
            dict(route=route, up=ffn_up, down=ffn_down)[task]()

    step = pl.program_id(0)
    for i, stage in enumerate(STAGES):
        @pl.when(step * (i + 2) < 1)
        def _(stage=stage):
            clock[2] = 0
            for phase in stage.split(" . "):
                clock[:2] = [0, NT * sum(t[0] in "qkvMT" for t in phase.split())]
                for task in phase.split() + ["."]:
                    run(task)
            while fillers:
                fillers.pop(0)()


@jax.jit
def pallas_gated_mix__sliding_local_dilated__moe_arch_mod__prompt_kernel(
    A_x, A_wqkv, A_wo, B_x, B_w_r, B_w_gate, B_w_up, B_w_down, gate_w,
):
    del B_x
    hbm = pl.BlockSpec(memory_space=pl.ANY)
    vm = pltpu.VMEM
    out = pl.pallas_call(
        _kernel,
        grid=(2,),
        in_specs=[hbm] * 8,
        out_specs=hbm,
        out_shape=jax.ShapeDtypeStruct((S, D), bf16),
        scratch_shapes=[
            vm((S // 2, D), u32), [vm((D, D), bf16)] * 3, vm((D, D), bf16), vm((D,), bf16), vm((D,), bf16),
            vm((F, D), bf16), vm((F, D), bf16), vm((F, D), bf16),
            [vm((NT, D // 2 + 16, 128), u32)] * 4, [vm((D // 2, D), u32)] * 3, vm((D // 2, D), u32),
            [[vm((NT, BM, 128), f32), vm((NT, HALO + BM, 128), f32), vm((NT, HALO + BM, 128), f32)]] * NB,
            [vm((BM // 2, D), u32)] * NB, vm((S, D), bf16), vm((16, F), bf16),
            [vm((BM, 128), f32)] * NB, [vm((NT, BM, 128), f32)] * NB, [vm((16, 128), f32)] * NB,
            vm((16, D), f32), vm((16, D), f32), vm((16, 128), f32), pltpu.SMEM((2,), i32),
            pltpu.SemaphoreType.DMA((len(COPIES),)),
        ],
        compiler_params=pltpu.CompilerParams(vmem_limit_bytes=100 * 2 ** 20, flags=FLAGS,
                                             dimension_semantics=("arbitrary",)),
    )(A_x.reshape(S, D), A_wqkv, A_wo, B_w_r, B_w_gate.T, B_w_up.T, B_w_down, gate_w)
    return out.reshape(A_x.shape)
```

```python
import functools

import jax
import jax.numpy as jnp
from jax import lax
import jax.experimental.pallas as pl
import jax.experimental.pallas.tpu as pltpu

S, D, F = 2048, 640, 1728
H, DH, WIN, DIL = 32, 20, 8, 2
NT = D // 128
HALO = 16
BM = 256
NB = S // BM
R = 8
EXP2_SCALE = (DH ** -0.5) * 1.4426950408889634
MASKED = -1e9 * 1.4426950408889634

STAGES = (
    "+q02 +q34 +x00 +x13 +gw +wr +k04 +v04 -q02 Wq02 -q34 Wq34 -x00 q0",
    "-x13 -gw -wr G0 G1 q1 q2",
    "-k04 -v04 +wo +x47 +wg G2 R3 Wk04 q3 Wv04 k0 v0",
    "-x47 +wu +wd R4 R5 R6 R7 . A0 k1 v1 k2",
    "K3 K4 A1 v2 k3 v3",
    "-wg -wu -wo route Wo q4 . up A2 k4 v4 q5 . A3 M0 k5 v5",
    "-wd down K5 K6 K7 A4 q6 k6 v6 . A5 M1 q7 k7",
    "O01 A6 v7 M2 M3 . O23 A74 M4 O44 M5 O55 M6 . O66 T7 -O01 -O23 -O44 -O55 -O66 -T70 -T71 -T72 -T73 -T74",
)
COPIES = [t[1:] for stage in STAGES for t in stage.split() if t[0] == "-"]
assert all(t[1:] in COPIES for stage in STAGES for t in stage.split() if t[0] == "+")
FLAGS = {"XLA_TPU_EVENLY_DISTRIBUTE_CRITICAL_NODES": True}
_NT_DIMS = (((1,), (1,)), ((), ()))
f32, bf16, u32, i32 = jnp.float32, jnp.bfloat16, jnp.uint32, jnp.int32


def _lanes(t):
    return slice(t * 128, (t + 1) * 128)


def _tree(op, xs):
    while len(xs) > 1:
        xs = [op(xs[i], xs[i + 1]) for i in range(0, len(xs), 2)]
    return xs[0]


def _sigmoid(z):
    return 1.0 / (1.0 + jnp.exp(-z))


def _kernel(x_hbm, wqkv_hbm, wo_hbm, wr_hbm, wg_hbm, wu_hbm, wd_hbm, gw_hbm, out_hbm,
            x_v, wqkv_v, wo_v, wr_v, gw_v, wg_v, wu_v, wd_v,
            words, wt_s, wop_s, qkv_s, o_bufs, out_s, h_s, g_s, keep_s, score_s, xs_s, ys_s, top_s, idx_s, sems):
    def rows(a, b):
        return pl.ds(a, b - a)

    def endpoints(name):
        if name[0] in "xO":
            r = rows(int(name[1]) * BM, (int(name[2]) + 1) * BM)
            if name[0] == "O":
                return out_s.at[r], out_hbm.at[r]
            r = rows(int(name[1]) * BM // 2, (int(name[2]) + 1) * BM // 2)
            return x_hbm.bitcast(u32).at[r], x_v.at[r]
        if name[0] == "T":
            r, c = pl.ds(int(name[1]) * BM, BM), pl.ds(int(name[2]) * 128, 128)
            return out_s.at[r, c], out_hbm.at[r, c]
        if name[0] in "qkv":
            p, r = "qkv".index(name[0]), rows(int(name[1]) * 128, (int(name[2]) + 1) * 128)
            return wqkv_hbm.at[r, pl.ds(p * D, D)], wqkv_v[p].at[r]
        return dict(wo=(wo_hbm, wo_v), wr=(wr_hbm, wr_v), gw=(gw_hbm, gw_v),
                    wg=(wg_hbm, wg_v), wu=(wu_hbm, wu_v), wd=(wd_hbm, wd_v))[name]

    copies = {name: pltpu.make_async_copy(*endpoints(name), sems.at[i]) for i, name in enumerate(COPIES)}

    def x_rows(r0, n, cols=slice(None)):
        return pltpu.bitcast(x_v[pl.ds(r0 // 2, n // 2), cols], bf16)

    def permute_rows(src_words, dst, t):
        for j in range(DH // 2):
            w = src_words[pl.ds(j, H, stride=DH // 2), :]
            lo = pltpu.bitcast(w << 16, f32).astype(bf16)
            hi = pltpu.bitcast(w & jnp.uint32(0xFFFF0000), f32).astype(bf16)
            dst[pl.ds(j * H, H // 2), _lanes(t)] = pltpu.bitcast(lo, u32)
            dst[pl.ds(j * H + H // 2, H // 2), _lanes(t)] = pltpu.bitcast(hi, u32)

    def prep_qkv(p, lo, hi):
        for t in range(lo, hi + 1):
            wt = wqkv_v[p][_lanes(t), :].T
            words[p][t, pl.ds(0, D // 2), :] = pltpu.bitcast(wt, u32)
            permute_rows(words[p].at[t], wt_s[p], t)

    def prep_wo():
        for t in range(NT):
            words[3][t, pl.ds(0, D // 2), :] = pltpu.bitcast(wo_v[:, _lanes(t)], u32)
            yield
            yield permute_rows(words[3].at[t], wop_s, t)

    fillers = []

    paced = []
    clock = [0, 0, 0]

    def matmul(tile):
        y = None
        for k in range(NT):
            y = tile(k) if y is None else y + tile(k)
            clock[2] += 1
            if clock[2] % 4 == 0 and k > 0:
                for _ in range(min(4, len(fillers))):
                    fillers.pop(0)()
        clock[0] += 1
        for item in paced:
            gen, total, done, slack = item
            item[2] = min(total, -(-total * clock[0] // max(clock[1] - slack, 1)))
            for _ in range(item[2] - done):
                next(gen)
        return y

    def proj(b, p):
        cur = qkv_s[b][p]
        for t in range(NT):
            yt = matmul(lambda k: lax.dot_general(
                x_rows(b * BM, BM, _lanes(k)), pltpu.bitcast(wt_s[p][pl.ds(t * 64, 64), _lanes(k)], bf16),
                _NT_DIMS, preferred_element_type=f32))
            if p == 0:
                cur[t] = yt
                continue
            cur[t, pl.ds(HALO, BM), :] = yt
            if b == 0:
                cur[t, pl.ds(0, HALO), :] = (jnp.zeros((HALO, 128), f32) if p == 1 else
                                             jnp.broadcast_to(yt[0:1], (HALO, 128)))
            if b + 1 < NB:
                qkv_s[b + 1][p][t, pl.ds(0, HALO), :] = yt[BM - HALO:]

    def attend(b):
        q_s, k_s, v_s = qkv_s[b]
        o_s = o_bufs[b]

        def scores(i):
            q = [q_s[t, pl.ds(i * R, R), :] * EXP2_SCALE for t in range(NT)]
            out = []
            for w in range(WIN):
                base = HALO + i * R - DIL * w
                s = q[0] * k_s[0, pl.ds(base, R), :]
                for t in range(1, NT):
                    s = s + q[t] * k_s[t, pl.ds(base, R), :]
                out.append((s, pltpu.roll(s, 64, 1)))
            return out

        def fold(parts):
            out = []
            for s, r in parts:
                s = s + r
                out.append((s, pltpu.roll(s, 32, 1)))
            return out

        def softmax(i, parts):
            logits = []
            for w, (s, r) in enumerate(parts):
                s = s + r
                if b * BM + i * R < DIL * w:
                    pos = b * BM + i * R + lax.broadcasted_iota(i32, (R, 128), 0)
                    s = jnp.where(pos >= DIL * w, s, MASKED)
                logits.append(s)
            m = _tree(jnp.maximum, logits)
            e = [jnp.exp2(s - m) for s in logits]
            den = _tree(jnp.add, e)
            return e, den, pl.reciprocal(den, approx=True)

        def values(i, parts):
            e, den, inv = parts
            inv = inv * (2.0 - den * inv)
            out = []
            for t in range(NT):
                acc = e[0] * v_s[t, pl.ds(HALO + i * R, R), :]
                for w in range(1, WIN):
                    acc = acc + e[w] * v_s[t, pl.ds(HALO + i * R - DIL * w, R), :]
                out.append(acc * inv)
            return out

        n = BM // R
        st = [{} for _ in range(4)]
        for c in range(n + 3):
            if c < n:
                st[0][c] = scores(c)
            if 0 <= c - 1 < n:
                st[1][c - 1] = fold(st[0].pop(c - 1))
            if 0 <= c - 2 < n:
                st[2][c - 2] = softmax(c - 2, st[1].pop(c - 2))
            if 0 <= c - 3 < n:
                i = c - 3
                st[3][i] = values(i, st[2].pop(i))
                if i % 2:
                    lo, hi = st[3].pop(i - 1), st[3].pop(i)
                    for t in range(NT):
                        o = jnp.concatenate([lo[t], hi[t]], axis=0).astype(bf16)
                        o_s[pl.ds((i - 1) * R // 2, R), _lanes(t)] = pltpu.bitcast(o, u32)
            yield

    def row_dot(x, w):
        s = x[:, _lanes(0)] * w[:, _lanes(0)]
        for t in range(1, NT):
            s = s + x[:, _lanes(t)] * w[:, _lanes(t)]
        return jnp.sum(s, axis=1, keepdims=True)

    def vec(ref):
        return ref[...].astype(f32).reshape(1, D)

    def mix(b, tiled_out=False):
        for t in range(NT):
            a = matmul(lambda k: jnp.dot(
                pltpu.bitcast(o_bufs[b][:, _lanes(k)], bf16),
                pltpu.bitcast(wop_s[pl.ds(k * 64, 64), _lanes(t)], bf16), preferred_element_type=f32))
            out_s[pl.ds(b * BM, BM), _lanes(t)] = (g_s[b][...] * a + keep_s[b][t]).astype(bf16)
            if tiled_out:
                patch(b * BM, (b + 1) * BM, _lanes(t))
                copies[f"T{b}{t}"].start()

    def gates(b, mixing, routing):
        gw, wr = vec(gw_v), vec(wr_v)
        lane = lax.broadcasted_iota(i32, (16, 128), 1)
        acc = jnp.zeros((16, 128), f32)
        for i in range(BM // 16):
            x = x_rows(b * BM + i * 16, 16).astype(f32)
            if mixing:
                g = _sigmoid(row_dot(x, gw))
                g_s[b][pl.ds(i * 16, 16), :] = jnp.broadcast_to(g, (16, 128))
                for t in range(NT):
                    keep_s[b][t, pl.ds(i * 16, 16), :] = (1.0 - g) * x[:, _lanes(t)]
            if routing:
                acc = jnp.where(lane == b * (BM // 16) + i, row_dot(x, wr), acc)
                if i == BM // 16 - 1:
                    score_s[b][...] = acc
            if i % 2:
                yield

    def route():
        lane = lax.broadcasted_iota(i32, (16, 128), 1)
        acc = score_s[0][...]
        for b in range(1, NB):
            acc = jnp.where(lane >= b * (BM // 16), score_s[b][...], acc)
        score = acc.astype(bf16).astype(f32)
        pos = lane * 16 + lax.broadcasted_iota(i32, (16, 128), 0)

        def best(sc, taken):
            top = jnp.max(jnp.max(sc, axis=1, keepdims=True), axis=0, keepdims=True)
            cand = jnp.where((sc == top) & (pos != taken), pos, S - 1)
            return top, jnp.min(jnp.min(cand, axis=1, keepdims=True), axis=0, keepdims=True)

        r1, p1 = best(score, -1)
        r2, p2 = best(jnp.where(pos == p1, -jnp.inf, score), p1)
        idx, top = (p1[0, 0], p2[0, 0]), (r1, r2)
        idx_s[0] = idx[0]
        idx_s[1] = idx[1]
        first = lax.broadcasted_iota(i32, (16, 128), 0) == 0
        top_s[...] = jnp.where(first, top[0], top[1])
        xs = gather(idx)
        xs_s[...] = xs

    def group(idx, lo, hi):
        return pl.multiple_of(jnp.clip(idx // 16, lo // 16, hi // 16 - 1) * 16, 16)

    def gather(idx):
        sel = []
        for j in range(2):
            g0 = group(idx[j], 0, S)
            xg = pltpu.bitcast(x_v[pl.ds(pl.multiple_of(g0 // 2, 8), 8), :], bf16).astype(f32)
            hit = lax.broadcasted_iota(i32, (16, D), 0) == idx[j] - g0
            sel.append(jnp.sum(jnp.where(hit, xg, 0.0), axis=0, keepdims=True))
        first = lax.broadcasted_iota(i32, (16, D), 0) == 0
        return jnp.where(first, sel[0], sel[1])

    f_tiles = [(n, min(128, F - n)) for n in range(0, F, 128)]

    def ffn_up():
        xb = xs_s[...].astype(bf16)
        acc = {}

        def tile(w_v, n, w, k):
            y = lax.dot_general(xb[:, _lanes(k)], w_v[pl.ds(n, w), _lanes(k)], _NT_DIMS, preferred_element_type=f32)
            key = w_v is wu_v
            acc[key] = y if k == 0 else acc[key] + y
            if key and k == NT - 1:
                g = acc[False]
                h_s[:, pl.ds(n, w)] = (g * _sigmoid(g) * acc[True]).astype(bf16)

        for n, w in f_tiles:
            for w_v in (wg_v, wu_v):
                fillers.extend(functools.partial(tile, w_v, n, w, k) for k in range(NT))

    def ffn_down():
        acc = {}

        def tile(t, n, w):
            y = jnp.dot(h_s[:, pl.ds(n, w)], wd_v[pl.ds(n, w), _lanes(t)], preferred_element_type=f32)
            acc[t] = y if n == 0 else acc[t] + y
            if n + w == F:
                ys_s[:, _lanes(t)] = acc[t] * scale

        gate = _sigmoid(row_dot(xs_s[...], vec(gw_v)))
        scale = _sigmoid(top_s[...]) * (1.0 - gate)
        for t in range(NT):
            fillers.extend(functools.partial(tile, t, n, w) for n, w in f_tiles)

    def patch(lo, hi, cols=slice(0, D)):
        idx, delta = (idx_s[0], idx_s[1]), ys_s[:, cols]
        for j in range(2):
            g0 = group(idx[j], lo, hi)
            hit = lax.broadcasted_iota(i32, (16, cols.stop - cols.start), 0) == idx[j] - g0
            cur = out_s[pl.ds(g0, 16), cols].astype(f32)
            out_s[pl.ds(g0, 16), cols] = jnp.where(hit, cur + delta[j:j + 1, :], cur).astype(bf16)

    def run(task):
        if task == ".":
            for gen, *_ in paced:
                for _ in gen:
                    pass
            paced.clear()
        elif task[0] == "+":
            copies[task[1:]].start()
        elif task[0] == "-":
            copies[task[1:]].wait()
        elif task[0] in "qkv":
            proj(int(task[1]), "qkv".index(task[0]))
        elif task[0] in "GKR":
            paced.append([gates(int(task[1]), task[0] != "R", task[0] != "K"), BM // 32, 0, int(task[2:] or 0)])
        elif task[0] == "A":
            paced.append([attend(int(task[1])), BM // R + 3, 0, int(task[2:] or 0)])
        elif task[0] in "MT":
            mix(int(task[1]), task[0] == "T")
        elif task[0] == "W":
            if task[1] == "o":
                paced.append([prep_wo(), 2 * NT, 0, 0])
            else:
                prep_qkv("qkv".index(task[1]), int(task[2]), int(task[3]))
        elif task[0] == "O":
            patch(int(task[1]) * BM, (int(task[2]) + 1) * BM)
            copies[task].start()
        else:
            dict(route=route, up=ffn_up, down=ffn_down)[task]()

    step = pl.program_id(0)

    @pl.when(step < 1)
    def _():
        for i, stage in enumerate(STAGES):
            @pl.when(step * (i + 2) < 1)
            def _(stage=stage):
                clock[2] = 0
                for phase in stage.split(" . "):
                    clock[:2] = [0, NT * sum(t[0] in "qkvMT" for t in phase.split())]
                    for task in phase.split() + ["."]:
                        run(task)
                while fillers:
                    fillers.pop(0)()


@jax.jit
def pallas_gated_mix__sliding_local_dilated__moe_arch_mod__prompt_kernel(
    A_x, A_wqkv, A_wo, B_x, B_w_r, B_w_gate, B_w_up, B_w_down, gate_w,
):
    del B_x
    hbm = pl.BlockSpec(memory_space=pl.ANY)
    vm = pltpu.VMEM
    out = pl.pallas_call(
        _kernel,
        grid=(2,),
        in_specs=[hbm] * 8,
        out_specs=hbm,
        out_shape=jax.ShapeDtypeStruct((S, D), bf16),
        scratch_shapes=[
            vm((S // 2, D), u32), [vm((D, D), bf16)] * 3, vm((D, D), bf16), vm((D,), bf16), vm((D,), bf16),
            vm((F, D), bf16), vm((F, D), bf16), vm((F, D), bf16),
            [vm((NT, D // 2 + 16, 128), u32)] * 4, [vm((D // 2, D), u32)] * 3, vm((D // 2, D), u32),
            [[vm((NT, BM, 128), f32), vm((NT, HALO + BM, 128), f32), vm((NT, HALO + BM, 128), f32)]] * NB,
            [vm((BM // 2, D), u32)] * NB, vm((S, D), bf16), vm((16, F), bf16),
            [vm((BM, 128), f32)] * NB, [vm((NT, BM, 128), f32)] * NB, [vm((16, 128), f32)] * NB,
            vm((16, D), f32), vm((16, D), f32), vm((16, 128), f32), pltpu.SMEM((2,), i32),
            pltpu.SemaphoreType.DMA((len(COPIES),)),
        ],
        compiler_params=pltpu.CompilerParams(vmem_limit_bytes=100 * 2 ** 20, flags=FLAGS,
                                             dimension_semantics=("arbitrary",)),
    )(A_x.reshape(S, D), A_wqkv, A_wo, B_w_r, B_w_gate.T, B_w_up.T, B_w_down, gate_w)
    return out.reshape(A_x.shape)
```

```python
import functools

import jax
import jax.numpy as jnp
from jax import lax
import jax.experimental.pallas as pl
import jax.experimental.pallas.tpu as pltpu

S, D, F = 2048, 640, 1728
H, DH, WIN, DIL = 32, 20, 8, 2
NT = D // 128
HALO = 16
BM = 256
NB = S // BM
R = 8
EXP2_SCALE = (DH ** -0.5) * 1.4426950408889634
MASKED = -1e9 * 1.4426950408889634

STAGES = (
    "+q02 +q34 +x00 +x13 +gw +wr +k04 +v04 -q02 Wq02 -q34 Wq34 -x00 q0",
    "-x13 -gw -wr G0 G1 q1 q2",
    "-k04 -v04 +wo +x47 +wg G2 R3 Wk04 q3 Wv04 k0 v0",
    "-x47 +wu +wd R4 R5 R6 R7 . A0 k1 v1 k2",
    "K3 K4 A1 v2 k3 v3",
    "-wg -wu -wo route Wo q4 . up A2 k4 v4 q5 . A3 M0 k5 v5",
    "-wd down K5 K6 K7 A4 q6 k6 v6 . A5 M1 q7 k7",
    "O01 A6 v7 M2 M3 . O23 A74 M4 O44 M5 O55 M6 . O66 T7 -O01 -O23 -O44 -O55 -O66 -T70 -T71 -T72 -T73 -T74",
)
COPIES = [t[1:] for stage in STAGES for t in stage.split() if t[0] == "-"]
assert all(t[1:] in COPIES for stage in STAGES for t in stage.split() if t[0] == "+")
FLAGS = {"XLA_TPU_EVENLY_DISTRIBUTE_CRITICAL_NODES": True}
_NT_DIMS = (((1,), (1,)), ((), ()))
f32, bf16, u32, i32 = jnp.float32, jnp.bfloat16, jnp.uint32, jnp.int32


def _lanes(t):
    return slice(t * 128, (t + 1) * 128)


def _tree(op, xs):
    while len(xs) > 1:
        xs = [op(xs[i], xs[i + 1]) for i in range(0, len(xs), 2)]
    return xs[0]


def _sigmoid(z):
    return 1.0 / (1.0 + jnp.exp(-z))


def _kernel(x_hbm, wqkv_hbm, wo_hbm, wr_hbm, wg_hbm, wu_hbm, wd_hbm, gw_hbm, out_hbm,
            x_v, wqkv_v, wo_v, wr_v, gw_v, wg_v, wu_v, wd_v,
            words, wt_s, wop_s, qkv_s, o_bufs, out_s, h_s, g_s, keep_s, score_s, xs_s, ys_s, top_s, idx_s, sems):
    def rows(a, b):
        return pl.ds(a, b - a)

    def endpoints(name):
        if name[0] in "xO":
            r = rows(int(name[1]) * BM, (int(name[2]) + 1) * BM)
            if name[0] == "O":
                return out_s.at[r], out_hbm.at[r]
            r = rows(int(name[1]) * BM // 2, (int(name[2]) + 1) * BM // 2)
            return x_hbm.bitcast(u32).at[r], x_v.at[r]
        if name[0] == "T":
            r, c = pl.ds(int(name[1]) * BM, BM), pl.ds(int(name[2]) * 128, 128)
            return out_s.at[r, c], out_hbm.at[r, c]
        if name[0] in "qkv":
            p, r = "qkv".index(name[0]), rows(int(name[1]) * 128, (int(name[2]) + 1) * 128)
            return wqkv_hbm.at[r, pl.ds(p * D, D)], wqkv_v[p].at[r]
        return dict(wo=(wo_hbm, wo_v), wr=(wr_hbm, wr_v), gw=(gw_hbm, gw_v),
                    wg=(wg_hbm.bitcast(u32), wg_v), wu=(wu_hbm.bitcast(u32), wu_v),
                    wd=(wd_hbm.bitcast(u32), wd_v))[name]

    copies = {name: pltpu.make_async_copy(*endpoints(name), sems.at[i]) for i, name in enumerate(COPIES)}

    def x_rows(r0, n, cols=slice(None)):
        return pltpu.bitcast(x_v[pl.ds(r0 // 2, n // 2), cols], bf16)

    def permute_rows(src_words, dst, t):
        for j in range(DH // 2):
            w = src_words[pl.ds(j, H, stride=DH // 2), :]
            lo = pltpu.bitcast(w << 16, f32).astype(bf16)
            hi = pltpu.bitcast(w & jnp.uint32(0xFFFF0000), f32).astype(bf16)
            dst[pl.ds(j * H, H // 2), _lanes(t)] = pltpu.bitcast(lo, u32)
            dst[pl.ds(j * H + H // 2, H // 2), _lanes(t)] = pltpu.bitcast(hi, u32)

    def prep_qkv(p, lo, hi):
        for t in range(lo, hi + 1):
            wt = wqkv_v[p][_lanes(t), :].T
            words[p][t, pl.ds(0, D // 2), :] = pltpu.bitcast(wt, u32)
            permute_rows(words[p].at[t], wt_s[p], t)

    def prep_wo():
        for t in range(NT):
            words[3][t, pl.ds(0, D // 2), :] = pltpu.bitcast(wo_v[:, _lanes(t)], u32)
            yield
            yield permute_rows(words[3].at[t], wop_s, t)

    fillers = []

    paced = []
    clock = [0, 0, 0]

    def matmul(tile):
        y = None
        for k in range(NT):
            y = tile(k) if y is None else y + tile(k)
            clock[2] += 1
            if clock[2] % 4 == 0 and k > 0:
                for _ in range(min(4, len(fillers))):
                    fillers.pop(0)()
        clock[0] += 1
        for item in paced:
            gen, total, done, slack = item
            item[2] = min(total, -(-total * clock[0] // max(clock[1] - slack, 1)))
            for _ in range(item[2] - done):
                next(gen)
        return y

    def proj(b, p):
        cur = qkv_s[b][p]
        for t in range(NT):
            yt = matmul(lambda k: lax.dot_general(
                x_rows(b * BM, BM, _lanes(k)), pltpu.bitcast(wt_s[p][pl.ds(t * 64, 64), _lanes(k)], bf16),
                _NT_DIMS, preferred_element_type=f32))
            if p == 0:
                cur[t] = yt
                continue
            cur[t, pl.ds(HALO, BM), :] = yt
            if b == 0:
                cur[t, pl.ds(0, HALO), :] = (jnp.zeros((HALO, 128), f32) if p == 1 else
                                             jnp.broadcast_to(yt[0:1], (HALO, 128)))
            if b + 1 < NB:
                qkv_s[b + 1][p][t, pl.ds(0, HALO), :] = yt[BM - HALO:]

    def attend(b):
        q_s, k_s, v_s = qkv_s[b]
        o_s = o_bufs[b]

        def scores(i):
            q = [q_s[t, pl.ds(i * R, R), :] * EXP2_SCALE for t in range(NT)]
            out = []
            for w in range(WIN):
                base = HALO + i * R - DIL * w
                s = q[0] * k_s[0, pl.ds(base, R), :]
                for t in range(1, NT):
                    s = s + q[t] * k_s[t, pl.ds(base, R), :]
                out.append((s, pltpu.roll(s, 64, 1)))
            return out

        def fold(parts):
            out = []
            for s, r in parts:
                s = s + r
                out.append((s, pltpu.roll(s, 32, 1)))
            return out

        def softmax(i, parts):
            logits = []
            for w, (s, r) in enumerate(parts):
                s = s + r
                if b * BM + i * R < DIL * w:
                    pos = b * BM + i * R + lax.broadcasted_iota(i32, (R, 128), 0)
                    s = jnp.where(pos >= DIL * w, s, MASKED)
                logits.append(s)
            m = _tree(jnp.maximum, logits)
            e = [jnp.exp2(s - m) for s in logits]
            den = _tree(jnp.add, e)
            return e, den, pl.reciprocal(den, approx=True)

        def values(i, parts):
            e, den, inv = parts
            inv = inv * (2.0 - den * inv)
            out = []
            for t in range(NT):
                acc = e[0] * v_s[t, pl.ds(HALO + i * R, R), :]
                for w in range(1, WIN):
                    acc = acc + e[w] * v_s[t, pl.ds(HALO + i * R - DIL * w, R), :]
                out.append(acc * inv)
            return out

        n = BM // R
        st = [{} for _ in range(4)]
        for c in range(n + 3):
            if c < n:
                st[0][c] = scores(c)
            if 0 <= c - 1 < n:
                st[1][c - 1] = fold(st[0].pop(c - 1))
            if 0 <= c - 2 < n:
                st[2][c - 2] = softmax(c - 2, st[1].pop(c - 2))
            if 0 <= c - 3 < n:
                i = c - 3
                st[3][i] = values(i, st[2].pop(i))
                if i % 2:
                    lo, hi = st[3].pop(i - 1), st[3].pop(i)
                    for t in range(NT):
                        o = jnp.concatenate([lo[t], hi[t]], axis=0).astype(bf16)
                        o_s[pl.ds((i - 1) * R // 2, R), _lanes(t)] = pltpu.bitcast(o, u32)
            yield

    def row_dot(x, w):
        s = x[:, _lanes(0)] * w[:, _lanes(0)]
        for t in range(1, NT):
            s = s + x[:, _lanes(t)] * w[:, _lanes(t)]
        return jnp.sum(s, axis=1, keepdims=True)

    def vec(ref):
        return ref[...].astype(f32).reshape(1, D)

    def mix(b, tiled_out=False):
        for t in range(NT):
            a = matmul(lambda k: jnp.dot(
                pltpu.bitcast(o_bufs[b][:, _lanes(k)], bf16),
                pltpu.bitcast(wop_s[pl.ds(k * 64, 64), _lanes(t)], bf16), preferred_element_type=f32))
            out_s[pl.ds(b * BM, BM), _lanes(t)] = (g_s[b][...] * a + keep_s[b][t]).astype(bf16)
            if tiled_out:
                patch(b * BM, (b + 1) * BM, _lanes(t))
                copies[f"T{b}{t}"].start()

    def gates(b, mixing, routing):
        gw, wr = vec(gw_v), vec(wr_v)
        lane = lax.broadcasted_iota(i32, (16, 128), 1)
        acc = jnp.zeros((16, 128), f32)
        for i in range(BM // 16):
            x = x_rows(b * BM + i * 16, 16).astype(f32)
            if mixing:
                g = _sigmoid(row_dot(x, gw))
                g_s[b][pl.ds(i * 16, 16), :] = jnp.broadcast_to(g, (16, 128))
                for t in range(NT):
                    keep_s[b][t, pl.ds(i * 16, 16), :] = (1.0 - g) * x[:, _lanes(t)]
            if routing:
                acc = jnp.where(lane == b * (BM // 16) + i, row_dot(x, wr), acc)
                if i == BM // 16 - 1:
                    score_s[b][...] = acc
            if i % 2:
                yield

    def route():
        lane = lax.broadcasted_iota(i32, (16, 128), 1)
        acc = score_s[0][...]
        for b in range(1, NB):
            acc = jnp.where(lane >= b * (BM // 16), score_s[b][...], acc)
        score = acc.astype(bf16).astype(f32)
        pos = lane * 16 + lax.broadcasted_iota(i32, (16, 128), 0)

        def best(sc, taken):
            top = jnp.max(jnp.max(sc, axis=1, keepdims=True), axis=0, keepdims=True)
            cand = jnp.where((sc == top) & (pos != taken), pos, S - 1)
            return top, jnp.min(jnp.min(cand, axis=1, keepdims=True), axis=0, keepdims=True)

        r1, p1 = best(score, -1)
        r2, p2 = best(jnp.where(pos == p1, -jnp.inf, score), p1)
        idx, top = (p1[0, 0], p2[0, 0]), (r1, r2)
        idx_s[0] = idx[0]
        idx_s[1] = idx[1]
        first = lax.broadcasted_iota(i32, (16, 128), 0) == 0
        top_s[...] = jnp.where(first, top[0], top[1])
        xs = gather(idx)
        xs_s[...] = xs

    def group(idx, lo, hi):
        return pl.multiple_of(jnp.clip(idx // 16, lo // 16, hi // 16 - 1) * 16, 16)

    def gather(idx):
        sel = []
        for j in range(2):
            g0 = group(idx[j], 0, S)
            xg = pltpu.bitcast(x_v[pl.ds(pl.multiple_of(g0 // 2, 8), 8), :], bf16).astype(f32)
            hit = lax.broadcasted_iota(i32, (16, D), 0) == idx[j] - g0
            sel.append(jnp.sum(jnp.where(hit, xg, 0.0), axis=0, keepdims=True))
        first = lax.broadcasted_iota(i32, (16, D), 0) == 0
        return jnp.where(first, sel[0], sel[1])

    f_tiles = [(n, min(128, F - n)) for n in range(0, F, 128)]

    def ffn_up():
        xb = xs_s[...].astype(bf16)
        acc = {}

        def tile(w_v, n, w, k):
            wt = pltpu.bitcast(w_v[pl.ds(n // 2, w // 2), _lanes(k)], bf16)
            y = lax.dot_general(xb[:, _lanes(k)], wt, _NT_DIMS, preferred_element_type=f32)
            key = w_v is wu_v
            acc[key] = y if k == 0 else acc[key] + y
            if key and k == NT - 1:
                g = acc[False]
                h_s[:, pl.ds(n, w)] = (g * _sigmoid(g) * acc[True]).astype(bf16)

        for n, w in f_tiles:
            for w_v in (wg_v, wu_v):
                fillers.extend(functools.partial(tile, w_v, n, w, k) for k in range(NT))

    def ffn_down():
        acc = {}

        def tile(t, n, w):
            wd = pltpu.bitcast(wd_v[pl.ds(n // 2, w // 2), _lanes(t)], bf16)
            y = jnp.dot(h_s[:, pl.ds(n, w)], wd, preferred_element_type=f32)
            acc[t] = y if n == 0 else acc[t] + y
            if n + w == F:
                ys_s[:, _lanes(t)] = acc[t] * scale

        gate = _sigmoid(row_dot(xs_s[...], vec(gw_v)))
        scale = _sigmoid(top_s[...]) * (1.0 - gate)
        for t in range(NT):
            fillers.extend(functools.partial(tile, t, n, w) for n, w in f_tiles)

    def patch(lo, hi, cols=slice(0, D)):
        idx, delta = (idx_s[0], idx_s[1]), ys_s[:, cols]
        for j in range(2):
            g0 = group(idx[j], lo, hi)
            hit = lax.broadcasted_iota(i32, (16, cols.stop - cols.start), 0) == idx[j] - g0
            cur = out_s[pl.ds(g0, 16), cols].astype(f32)
            out_s[pl.ds(g0, 16), cols] = jnp.where(hit, cur + delta[j:j + 1, :], cur).astype(bf16)

    def run(task):
        if task == ".":
            for gen, *_ in paced:
                for _ in gen:
                    pass
            paced.clear()
        elif task[0] == "+":
            copies[task[1:]].start()
        elif task[0] == "-":
            copies[task[1:]].wait()
        elif task[0] in "qkv":
            proj(int(task[1]), "qkv".index(task[0]))
        elif task[0] in "GKR":
            paced.append([gates(int(task[1]), task[0] != "R", task[0] != "K"), BM // 32, 0, int(task[2:] or 0)])
        elif task[0] == "A":
            paced.append([attend(int(task[1])), BM // R + 3, 0, int(task[2:] or 0)])
        elif task[0] in "MT":
            mix(int(task[1]), task[0] == "T")
        elif task[0] == "W":
            if task[1] == "o":
                paced.append([prep_wo(), 2 * NT, 0, 0])
            else:
                prep_qkv("qkv".index(task[1]), int(task[2]), int(task[3]))
        elif task[0] == "O":
            patch(int(task[1]) * BM, (int(task[2]) + 1) * BM)
            copies[task].start()
        else:
            dict(route=route, up=ffn_up, down=ffn_down)[task]()

    step = pl.program_id(0)

    @pl.when(step < 1)
    def _():
        for i, stage in enumerate(STAGES):
            @pl.when(step * (i + 2) < 1)
            def _(stage=stage):
                clock[2] = 0
                for phase in stage.split(" . "):
                    clock[:2] = [0, NT * sum(t[0] in "qkvMT" for t in phase.split())]
                    for task in phase.split() + ["."]:
                        run(task)
                while fillers:
                    fillers.pop(0)()


@jax.jit
def pallas_gated_mix__sliding_local_dilated__moe_arch_mod__prompt_kernel(
    A_x, A_wqkv, A_wo, B_x, B_w_r, B_w_gate, B_w_up, B_w_down, gate_w,
):
    del B_x
    hbm = pl.BlockSpec(memory_space=pl.ANY)
    vm = pltpu.VMEM
    out = pl.pallas_call(
        _kernel,
        grid=(2,),
        in_specs=[hbm] * 8,
        out_specs=hbm,
        out_shape=jax.ShapeDtypeStruct((S, D), bf16),
        scratch_shapes=[
            vm((S // 2, D), u32), [vm((D, D), bf16)] * 3, vm((D, D), bf16), vm((D,), bf16), vm((D,), bf16),
            vm((F // 2, D), u32), vm((F // 2, D), u32), vm((F // 2, D), u32),
            [vm((NT, D // 2 + 16, 128), u32)] * 4, [vm((D // 2, D), u32)] * 3, vm((D // 2, D), u32),
            [[vm((NT, BM, 128), f32), vm((NT, HALO + BM, 128), f32), vm((NT, HALO + BM, 128), f32)]] * NB,
            [vm((BM // 2, D), u32)] * NB, vm((S, D), bf16), vm((16, F), bf16),
            [vm((BM, 128), f32)] * NB, [vm((NT, BM, 128), f32)] * NB, [vm((16, 128), f32)] * NB,
            vm((16, D), f32), vm((16, D), f32), vm((16, 128), f32), pltpu.SMEM((2,), i32),
            pltpu.SemaphoreType.DMA((len(COPIES),)),
        ],
        compiler_params=pltpu.CompilerParams(vmem_limit_bytes=100 * 2 ** 20, flags=FLAGS,
                                             dimension_semantics=("arbitrary",)),
    )(A_x.reshape(S, D), A_wqkv, A_wo, B_w_r, B_w_gate.T, B_w_up.T, B_w_down, gate_w)
    return out.reshape(A_x.shape)
```
